```python
import os as _os
_os.environ.setdefault("JAX_PLATFORMS", "cpu")
import jax
import jax.numpy as jnp

def _softmax(x, axis=-1):
    return jax.nn.softmax(x, axis=axis)
def _gelu(x):
    return jax.nn.gelu(x, approximate=True)
def _silu(x):
    return jax.nn.silu(x)
def _sigmoid(x):
    return jax.nn.sigmoid(x)
def _layernorm(x, axis=-1, eps=1e-5):
    m = jnp.mean(x, axis=axis, keepdims=True)
    v = jnp.var(x, axis=axis, keepdims=True)
    return (x - m) / jnp.sqrt(v + eps)
def _scatter_add(tgt, idx, src, axis=0):
    return tgt.at[idx].add(src)
def _segment_sum(src, seg, n):
    return jax.ops.segment_sum(src, seg, n)
class _Rng:
    def __init__(self, key):
        self._k = key
    def _next(self):
        self._k, sub = jax.random.split(self._k)
        return sub
    def normal(self, shape):
        return jax.random.normal(self._next(), shape, dtype=jnp.bfloat16)
    def randint(self, lo, hi, shape):
        return jax.random.randint(self._next(), shape, lo, hi, dtype=jnp.int32)
    def uniform(self, shape, lo=0.0, hi=1.0):
        return jax.random.uniform(self._next(), shape, jnp.bfloat16, lo, hi)
    def permutation(self, n):
        return jax.random.permutation(self._next(), n)


kernel_name = 'sequential_preLN__softmax_full_mha__glu_gated_swiglu__prompt'

def setup_inputs():
    _rng = _Rng(jax.random.key(int.from_bytes(__import__("os").urandom(4), "little")))
    _w = (lambda a: (lambda t: t.astype(jnp.bfloat16) if jnp.issubdtype(t.dtype, jnp.floating) else t)(jnp.asarray(a)))
    def _A_setup():
        B, S, D = 1, 2048, 512
        return {
            "x": _w((lambda *s: _rng.normal(s) * 0.05)(B, S, D)),
            "wqkv": _w((lambda *s: _rng.normal(s) * 0.05)(D, 3 * D)),
            "wo": _w((lambda *s: _rng.normal(s) * 0.05)(D, D)),
        }
    _A_in = _A_setup()

    def _B_setup():
        B, S, D, F = 1, 2048, 512, 1376
        return {
            "x": _w((lambda *s: _rng.normal(s) * 0.05)(B, S, D)),
            "w1": _w((lambda *s: _rng.normal(s) * 0.05)(D, F) * (2.0 / D) ** 0.5),
            "w3": _w((lambda *s: _rng.normal(s) * 0.05)(D, F) * (2.0 / D) ** 0.5),
            "w2": _w((lambda *s: _rng.normal(s) * 0.05)(F, D) * (2.0 / F) ** 0.5),
        }
    _B_in = _B_setup()

    return {
        "A_x": _A_in["x"],
        "A_wqkv": _A_in["wqkv"],
        "A_wo": _A_in["wo"],
        "B_x": _B_in["x"],
        "B_w1": _B_in["w1"],
        "B_w3": _B_in["w3"],
        "B_w2": _B_in["w2"],
    }

def reference(A_x, A_wqkv, A_wo, B_x, B_w1, B_w3, B_w2):
    def _A_ref(x, wqkv, wo):
        B, S, D = x.shape
        H = 32; Dh = D // H
        qkv = (lambda x, *d: x.transpose(*d))((x @ wqkv).reshape(B, S, 3, H, Dh), 2, 0, 3, 1, 4)
        q, k, v = qkv[0], qkv[1], qkv[2]
        scale = Dh ** -0.5
        scores = jnp.einsum("bhqd,bhkd->bhqk", q, k) * scale
        p = _softmax(scores, axis=-1)
        o = jnp.einsum("bhqk,bhkd->bhqd", p, v)
        return (lambda x, *d: x.transpose(*d))(o, 0, 2, 1, 3).reshape(B, S, D) @ wo

    def _B_ref(x, w1, w3, w2):
        gate = jnp.einsum("bsd,df->bsf", x, w1)
        up = jnp.einsum("bsd,df->bsf", x, w3)
        h = _silu(gate) * up
        out = jnp.einsum("bsf,fd->bsd", h, w2)
        return out

    x = A_x
    h = x + _A_ref(_layernorm(x, axis=-1), A_wqkv, A_wo)
    h2 = h + _B_ref(_layernorm(h, axis=-1), B_w1, B_w3, B_w2)
    return h2
```

```python
import jax
import jax.numpy as jnp
from jax import lax
from jax.experimental import pallas as pl
from jax.experimental.pallas import tpu as pltpu

S, D, H, DH, F = 2048, 512, 32, 16, 1376
LOG2E = 1.4426950408889634
EPS = 1e-5
f32, bf16 = jnp.float32, jnp.bfloat16
BQ = 512
NQ = S // BQ
C = 128
NC = S // C
NLT = BQ // 128
HPS = 2
NAS = H // HPS
L_LO, L_HI, A_HI = 2.0 ** -40, 2.0 ** 60, 2.0 ** 100
NT = (((1,), (1,)), ((), ()))


def _ln(x):
    m = jnp.mean(x, axis=-1, keepdims=True)
    xc = x - m
    v = jnp.mean(xc * xc, axis=-1, keepdims=True)
    return xc * lax.rsqrt(v + EPS)


def make(OFFB=2, FB=512, FSUB=1, FORCE_FALLBACK=0):
    BPC = C // 16
    NB = NC * BPC
    NF = S // FB

    def kern(x_hbm, wqkv_hbm, wo_hbm, w1t_hbm, w3t_hbm, w2_hbm, o_ref,
             x_v, wqkv_v, wo_v, w1t_v, w3t_v, w2_v,
             k_scr, qt_scr, vt_scr, ot_scr, bad_scr, sems):
        step = pl.program_id(0)

        def x_copy(i):
            return pltpu.make_async_copy(x_hbm.at[pl.ds(i * BQ, BQ), :], x_v.at[pl.ds(i * BQ, BQ), :], sems.at[i])

        def w_copy(j):
            return pltpu.make_async_copy(wqkv_hbm.at[:, pl.ds(j * D, D)], wqkv_v.at[:, pl.ds(j * D, D)], sems.at[NQ + j])

        late = [(wo_hbm, wo_v), (w1t_hbm, w1t_v), (w3t_hbm, w3t_v), (w2_hbm, w2_v)]

        def late_copy(j):
            return pltpu.make_async_copy(late[j][0], late[j][1], sems.at[NQ + 3 + j])

        def masked_qt(h, qb):
            g = h // 8
            qt = qt_scr[qb, pl.ds(pl.multiple_of(g * 128, 128), 128), :]
            rows = lax.broadcasted_iota(jnp.int32, (128, BQ), 0) // DH
            return jnp.where(rows == h % 8, qt.astype(f32), 0.0).astype(bf16)

        @pl.when(step == 0)
        def _():
            x_copy(0).start()
            w_copy(1).start()
            w_copy(0).start()
            w_copy(2).start()
            for i in range(1, NQ):
                x_copy(i).start()
            for j in range(4):
                late_copy(j).start()
            bad_scr[...] = jnp.zeros_like(bad_scr)
            wq_t = wv_t = None
            for qb in range(NQ):
                rows = pl.ds(qb * BQ, BQ)
                x_copy(qb).wait()
                xn = _ln(x_v[rows, :].astype(f32)).astype(bf16)
                if qb == 0:
                    w_copy(1).wait()
                k = jnp.dot(xn, wqkv_v[:, D:2 * D], preferred_element_type=f32).astype(bf16)
                for cc in range(BQ // C):
                    c = qb * (BQ // C) + cc
                    for b in range(BPC):
                        r0 = cc * C + (BPC - 1 - b) * 16
                        for g in range(4):
                            k_scr[g, pl.ds((c * BPC + b) * 16, 16), :] = k[r0:r0 + 16, g * 128:(g + 1) * 128]
                if qb == 0:
                    w_copy(0).wait()
                    wq_t = wqkv_v[:, 0:D].astype(f32).T.astype(bf16)
                qt = lax.dot_general(wq_t, xn, NT, preferred_element_type=f32)
                qt_scr[qb] = (qt * (DH ** -0.5 * LOG2E)).astype(bf16)
                if qb == 0:
                    w_copy(2).wait()
                    wv_t = wqkv_v[:, 2 * D:3 * D].astype(f32).T.astype(bf16)
                vt = lax.dot_general(wv_t, xn, NT, preferred_element_type=f32)
                vt_scr[:, :, rows] = vt.astype(bf16).reshape(H, DH, BQ)

        @pl.when(step < NAS)
        def _():
            h0 = step * HPS
            items = [(u, qb) for u in range(HPS) for qb in range(NQ)]
            NI = len(items)
            qms, blk, acc, lacc = {}, {}, {}, {}
            chunks = [(it, c) for it in range(NI) for c in range(NC)]
            bad = [None]

            def sum_add(it, p16, j):
                s2 = p16[0:8] + p16[8:16]
                key = (it, j % 2)
                lacc[key] = s2 if key not in lacc else lacc[key] + s2

            def emit_pv(ci):
                it, c = chunks[ci]
                u, qb = items[it]
                ps = []
                for b in range(BPC):
                    p16 = jnp.exp2(blk.pop((it, c * BPC + b)))
                    sum_add(it, p16, b)
                    ps.append(p16)
                p = jnp.concatenate(ps[::-1], axis=0).astype(bf16)
                vt = vt_scr[h0 + u, :, pl.ds(c * C, C)]
                pv = jnp.dot(vt, p, preferred_element_type=f32)
                acc[it] = pv if c == 0 else acc[it] + pv
                if c == NC - 1:
                    l = jnp.sum(lacc.pop((it, 0)) + lacc.pop((it, 1)), axis=0, keepdims=True)
                    a = acc.pop(it)
                    ok_l = jnp.logical_and(l >= L_LO, l <= L_HI)
                    ok_a = jnp.abs(a) <= A_HI
                    b_a = jnp.where(ok_a, 0.0, 1.0)
                    b_i = jnp.maximum(jnp.maximum(b_a[0:8], b_a[8:16]), jnp.where(ok_l, 0.0, 1.0))
                    bad[0] = b_i if bad[0] is None else jnp.maximum(bad[0], b_i)
                    o = a * (1.0 / l)
                    ot_scr[qb, pl.ds(pl.multiple_of((h0 + u) * DH, DH), DH), :] = o.astype(bf16)

            segs = []
            for it in range(NI):
                bounds = sorted(set([0, NB] + [c * BPC + OFFB for c in range(NC) if c * BPC + OFFB < NB]))
                for a, b in zip(bounds[:-1], bounds[1:]):
                    segs.append((it, a, b))
            pvi = 0
            for (it, a, b) in segs:
                u, qb = items[it]
                if a == 0:
                    qms[it] = masked_qt(h0 + u, qb)
                g = (h0 + u) // 8
                sm = jnp.dot(k_scr[g, pl.ds(a * 16, (b - a) * 16), :], qms[it], preferred_element_type=f32)
                for j in range(a, b):
                    blk[(it, j)] = sm[(j - a) * 16:(j - a + 1) * 16]
                pos = it * NB + b
                while pvi < len(chunks):
                    cit, cc = chunks[pvi]
                    if cit * NB + (cc + 2) * BPC + OFFB > pos:
                        break
                    emit_pv(pvi)
                    pvi += 1
            while pvi < len(chunks):
                emit_pv(pvi)
                pvi += 1
            bad_scr[...] = jnp.maximum(bad_scr[...], bad[0])

        @pl.when(step == NAS)
        def _():
            for j in range(4):
                late_copy(j).wait()
            flag = jnp.max(bad_scr[...]) > (-1.0 if FORCE_FALLBACK else 0.0)

            @pl.when(flag)
            def _():
                def body(i, carry):
                    h = i // NQ
                    qb = i % NQ
                    s = jnp.dot(k_scr[h // 8], masked_qt(h, qb), preferred_element_type=f32)
                    m = jnp.max(s, axis=0, keepdims=True)
                    p = jnp.exp2(s - m)
                    l = jnp.sum(p, axis=0, keepdims=True)
                    pn = jnp.concatenate(
                        [p[(c * BPC + BPC - 1 - b) * 16:(c * BPC + BPC - b) * 16] for c in range(NC) for b in range(BPC)],
                        axis=0).astype(bf16)
                    a = jnp.dot(vt_scr[h], pn, preferred_element_type=f32)
                    ot_scr[qb, pl.ds(pl.multiple_of(h * DH, DH), DH), :] = (a * (1.0 / l)).astype(bf16)
                    return carry
                lax.fori_loop(0, H * NQ, body, 0)

        @pl.when(step >= NAS)
        def _():
            fb = step - NAS
            sub = FB // FSUB
            for j in range(FSUB):
                r0 = pl.multiple_of(fb * FB + j * sub, sub)
                rows = pl.ds(r0, sub)
                qb = (fb * FB) // BQ
                col0 = (j * sub) if FB == BQ else None
                if FB == BQ:
                    ot = ot_scr[qb, :, pl.ds(j * sub, sub)]
                else:
                    raise NotImplementedError
                o = ot.astype(f32).T.astype(bf16)
                h1 = x_v[rows, :].astype(f32) + jnp.dot(o, wo_v[...], preferred_element_type=f32)
                hn = _ln(h1).astype(bf16)
                gate = lax.dot_general(hn, w1t_v[...], NT, preferred_element_type=f32)
                up = lax.dot_general(hn, w3t_v[...], NT, preferred_element_type=f32)
                a = (gate * jax.nn.sigmoid(gate) * up).astype(bf16)
                out = h1 + jnp.dot(a, w2_v[...], preferred_element_type=f32)
                o_ref[pl.ds(j * sub, sub), :] = out.astype(o_ref.dtype)

    @jax.jit
    def f(A_x, A_wqkv, A_wo, B_x, B_w1, B_w3, B_w2):
        x = A_x.reshape(S, D)
        hbm = pl.BlockSpec(memory_space=pl.ANY)
        out = pl.pallas_call(
            kern,
            grid=(NAS + NF,),
            in_specs=[hbm] * 6,
            out_specs=pl.BlockSpec((FB, D), lambda i: (jnp.maximum(i - NAS, 0), 0)),
            out_shape=jax.ShapeDtypeStruct((S, D), bf16),
            scratch_shapes=[
                pltpu.VMEM((S, D), bf16),
                pltpu.VMEM((D, 3 * D), bf16),
                pltpu.VMEM((D, D), bf16),
                pltpu.VMEM((F, D), bf16),
                pltpu.VMEM((F, D), bf16),
                pltpu.VMEM((F, D), bf16),
                pltpu.VMEM((4, NB * 16, 128), bf16),
                pltpu.VMEM((NQ, D, BQ), bf16),
                pltpu.VMEM((H, DH, S), bf16),
                pltpu.VMEM((NQ, D, BQ), bf16),
                pltpu.VMEM((8, BQ), f32),
                pltpu.SemaphoreType.DMA((NQ + 3 + 4,)),
            ],
            compiler_params=pltpu.CompilerParams(dimension_semantics=("arbitrary",), vmem_limit_bytes=100 * 1024 * 1024),
        )(x, A_wqkv, A_wo, B_w1.T, B_w3.T, B_w2)
        return out.reshape(1, S, D)
    return f


_kernel_fn = make()


@jax.jit
def pallas_sequential_preLN__softmax_full_mha__glu_gated_swiglu__prompt_kernel(
    A_x: jax.Array,
    A_wqkv: jax.Array,
    A_wo: jax.Array,
    B_x: jax.Array,
    B_w1: jax.Array,
    B_w3: jax.Array,
    B_w2: jax.Array,
):
    return _kernel_fn(A_x, A_wqkv, A_wo, B_x, B_w1, B_w3, B_w2)
```

```python
import jax
import jax.numpy as jnp
from jax import lax
from jax.experimental import pallas as pl
from jax.experimental.pallas import tpu as pltpu

S, D, H, DH, F = 2048, 512, 32, 16, 1376
LOG2E = 1.4426950408889634
EPS = 1e-5
f32, bf16 = jnp.float32, jnp.bfloat16

BQ = 512
NQ = S // BQ
NLT = BQ // 128
C = 128
NC = S // C
HPS = 2
NAS = H // HPS
OFFB = 2
VAHEAD = 5
VPAT = (16, 16, 0)
FSUB = 4
L_LO, L_HI, A_HI = 2.0 ** -40, 2.0 ** 60, 2.0 ** 100
NT = (((1,), (1,)), ((), ()))

RV = [VPAT[c % len(VPAT)] for c in range(NC)]
RM = [C - v for v in RV]
BPC = [r // 16 for r in RM]
MSTART = [sum(BPC[:c]) for c in range(NC + 1)]
VSTART = [sum(RV[:c]) for c in range(NC + 1)]
NB = MSTART[-1]
NBP = -(-NB // 4) * 4
NV = VSTART[-1]


def _ln(x):
    m = jnp.mean(x, axis=-1, keepdims=True)
    xc = x - m
    v = jnp.mean(xc * xc, axis=-1, keepdims=True)
    return xc * lax.rsqrt(v + EPS)


def _kernel(x_hbm, wqkv_hbm, wo_hbm, w1t_hbm, w3t_hbm, w2_hbm, o_ref,
            x_v, wqkv_v, wo_v, w1t_v, w3t_v, w2_v,
            k_scr, kv_scr, qt_scr, vt_scr, ot_scr, bad_scr, kb_a, kb_b, qb_a, qb_b, sems):
    step = pl.program_id(0)

    def x_copy(i):
        return pltpu.make_async_copy(x_hbm.at[pl.ds(i * BQ, BQ), :], x_v.at[pl.ds(i * BQ, BQ), :], sems.at[i])

    def w_copy(j):
        return pltpu.make_async_copy(wqkv_hbm.at[:, pl.ds(j * D, D)], wqkv_v.at[:, pl.ds(j * D, D)], sems.at[NQ + j])

    late = [(wo_hbm, wo_v), (w1t_hbm, w1t_v), (w3t_hbm, w3t_v), (w2_hbm, w2_v)]

    def late_copy(j):
        return pltpu.make_async_copy(late[j][0], late[j][1], sems.at[NQ + 3 + j])

    def masked_qt(h, qb):
        qt = qt_scr[qb, pl.ds(pl.multiple_of((h // 8) * 128, 128), 128), :]
        rows = lax.broadcasted_iota(jnp.int32, (128, BQ), 0) // DH
        return jnp.where(rows == h % 8, qt.astype(f32), 0.0).astype(bf16)

    def produce_kb(h, kb):
        x = pltpu.roll(kv_scr[h // 8], (128 - (h % 8) * DH) % 128, 1)
        for d in range(DH):
            kb[d] = jnp.broadcast_to(x[:, d:d + 1], (NV, 128))

    def prep_qb(h, qb, qbs):
        q16 = qt_scr[qb, pl.ds(pl.multiple_of(h * DH, DH), DH), :].astype(f32)
        for d in range(DH):
            qbs[d] = jnp.broadcast_to(q16[d:d + 1, :], (8, BQ))

    @pl.when(step == 0)
    def _():
        x_copy(0).start()
        w_copy(1).start()
        bad_scr[...] = jnp.zeros_like(bad_scr)

        def proj_k(qb, xn):
            k = jnp.dot(xn, wqkv_v[:, D:2 * D], preferred_element_type=f32).astype(bf16)
            for cc in range(BQ // C):
                c = qb * (BQ // C) + cc
                for b in range(BPC[c]):
                    r0 = cc * C + (BPC[c] - 1 - b) * 16
                    for g in range(4):
                        k_scr[g, pl.ds((MSTART[c] + b) * 16, 16), :] = k[r0:r0 + 16, g * 128:(g + 1) * 128]
                if RV[c]:
                    r0 = cc * C + RM[c]
                    kf = k[r0:r0 + RV[c]].astype(f32)
                    for g in range(4):
                        kv_scr[g, pl.ds(VSTART[c], RV[c]), :] = kf[:, g * 128:(g + 1) * 128]

        def proj_q(qb, xn, wq_t):
            qt = lax.dot_general(wq_t, xn, NT, preferred_element_type=f32)
            qt_scr[qb] = (qt * (DH ** -0.5 * LOG2E)).astype(bf16)

        def proj_v(qb, xn, wv_t):
            vt = lax.dot_general(wv_t, xn, NT, preferred_element_type=f32)
            vt_scr[:, :, pl.ds(qb * BQ, BQ)] = vt.astype(bf16).reshape(H, DH, BQ)

        def ln_chunk(qb):
            return _ln(x_v[pl.ds(qb * BQ, BQ), :].astype(f32)).astype(bf16)

        x_copy(0).wait()
        w_copy(0).start()
        xn0 = ln_chunk(0)
        w_copy(1).wait()
        w_copy(2).start()
        for i in range(1, NQ):
            x_copy(i).start()
        proj_k(0, xn0)
        w_copy(0).wait()
        wq_t = wqkv_v[:, 0:D].astype(f32).T.astype(bf16)
        proj_q(0, xn0, wq_t)
        for j in range(len(late)):
            late_copy(j).start()
        w_copy(2).wait()
        for i in range(1, NQ):
            x_copy(i).wait()
        wv_t = wqkv_v[:, 2 * D:3 * D].astype(f32).T.astype(bf16)
        proj_v(0, xn0, wv_t)
        for qb in range(1, NQ):
            xn = ln_chunk(qb)
            proj_k(qb, xn)
            proj_q(qb, xn, wq_t)
            proj_v(qb, xn, wv_t)
        produce_kb(0, kb_a)
        prep_qb(0, 0, qb_a)

    @pl.when(step < NAS)
    def _():
        h0 = step * HPS
        items = [(u, qb) for u in range(HPS) for qb in range(NQ)]
        kbs = [kb_a, kb_b]
        qbs_ = [qb_a, qb_b]
        qms, blk, acc, lacc, vout = {}, {}, {}, {}, {}
        chunks = [(it, c) for it in range(len(items)) for c in range(NC)]
        vpieces = [(it, c, lt, hf) for (it, c) in chunks if RV[c] for lt in range(NLT) for hf in range(2)]
        st = {"bad": None, "link": None, "vi": 0, "cur": None}

        def emit_vpiece():
            if st["vi"] >= len(vpieces):
                return
            it, c, lt, hf = vpieces[st["vi"]]
            st["vi"] += 1
            kb, qbs = kbs[items[it][0] % 2], qbs_[it % 2]
            if hf == 0:
                a = None if st["link"] is None else st["link"] - st["link"]
            else:
                a = st["cur"]
            for d in range(hf * 8, hf * 8 + 8):
                kbd = kb[d, pl.ds(VSTART[c], RV[c]), :]
                qbb = jnp.concatenate([qbs[d, :, pl.ds(lt * 128, 128)]] * (RV[c] // 8), axis=0)
                term = kbd * qbb
                a = term if a is None else a + term
            st["cur"] = a
            if hf == 1:
                vout.setdefault((it, c), []).append(a)
                st["link"] = a

        def prep_next(it):
            u, qb = items[it]
            h = h0 + u
            if qb == 0:
                produce_kb(jnp.minimum(h + 1, H - 1), kbs[(u + 1) % 2])
            if qb < NQ - 1:
                prep_qb(h, qb + 1, qbs_[(it + 1) % 2])
            else:
                prep_qb(jnp.minimum(h + 1, H - 1), 0, qbs_[(it + 1) % 2])

        def sum_add(it, p16, j):
            s2 = p16[0:8] + p16[8:16]
            key = (it, j % 2)
            lacc[key] = s2 if key not in lacc else lacc[key] + s2

        def emit_pv(ci):
            it, c = chunks[ci]
            u, qb = items[it]
            if c == 1:
                prep_next(it)
            while RV[c] and len(vout.get((it, c), [])) < NLT:
                emit_vpiece()
            target = len([cc for cc in chunks[:ci + 1 + VAHEAD] if RV[cc[1]]]) * NLT * 2
            todo = max(target - st["vi"], 0)
            ps = []
            if RV[c]:
                pvv = jnp.exp2(jnp.concatenate(vout.pop((it, c)), axis=1))
                sum_add(it, pvv, 0)
            for b in range(BPC[c]):
                p16 = jnp.exp2(blk.pop((it, MSTART[c] + b)))
                sum_add(it, p16, b + 1)
                ps.append(p16)
                for _ in range((todo * (b + 1)) // BPC[c] - (todo * b) // BPC[c]):
                    emit_vpiece()
            ps = ps[::-1]
            if RV[c]:
                ps.append(pvv)
            p = jnp.concatenate(ps, axis=0).astype(bf16)
            pv = jnp.dot(vt_scr[h0 + u, :, pl.ds(c * C, C)], p, preferred_element_type=f32)
            acc[it] = pv if c == 0 else acc[it] + pv
            if c == NC - 1:
                l = jnp.sum(lacc.pop((it, 0)) + lacc.pop((it, 1)), axis=0, keepdims=True)
                a = acc.pop(it)
                ok_l = jnp.logical_and(l >= L_LO, l <= L_HI)
                b_a = jnp.where(jnp.abs(a) <= A_HI, 0.0, 1.0)
                b_i = jnp.maximum(jnp.maximum(b_a[0:8], b_a[8:16]), jnp.where(ok_l, 0.0, 1.0))
                st["bad"] = b_i if st["bad"] is None else jnp.maximum(st["bad"], b_i)
                ot_scr[qb, pl.ds(pl.multiple_of((h0 + u) * DH, DH), DH), :] = (a * (1.0 / l)).astype(bf16)

        pvi = 0
        for it, (u, qb) in enumerate(items):
            qms[it] = masked_qt(h0 + u, qb)
            bounds = sorted(set([0, NB] + [MSTART[c] + OFFB for c in range(NC) if MSTART[c] + OFFB < NB]))
            for a, b in zip(bounds[:-1], bounds[1:]):
                sm = jnp.dot(k_scr[(h0 + u) // 8, pl.ds(a * 16, (b - a) * 16), :], qms[it], preferred_element_type=f32)
                for j in range(a, b):
                    blk[(it, j)] = sm[(j - a) * 16:(j - a + 1) * 16]
                pos = it * NB + b
                while pvi < len(chunks):
                    cit, cc = chunks[pvi]
                    nxt = cc + 2
                    need = cit * NB + MSTART[nxt] if nxt <= NC else (cit + 1) * NB + MSTART[nxt - NC]
                    if need + OFFB > pos:
                        break
                    emit_pv(pvi)
                    pvi += 1
        while pvi < len(chunks):
            emit_pv(pvi)
            pvi += 1
        bad_scr[...] = jnp.maximum(bad_scr[...], st["bad"])

    @pl.when(step == NAS)
    def _():
        for j in range(len(late)):
            late_copy(j).wait()

        @pl.when(jnp.max(bad_scr[...]) > 0.0)
        def _():
            def body(i, carry):
                h = i // NQ
                qb = i % NQ
                qm = masked_qt(h, qb)
                sm = jnp.dot(k_scr[h // 8, pl.ds(0, NB * 16), :], qm, preferred_element_type=f32)
                sv = jnp.dot(kv_scr[h // 8].astype(bf16), qm, preferred_element_type=f32)
                m = jnp.maximum(jnp.max(sm, axis=0, keepdims=True), jnp.max(sv, axis=0, keepdims=True))
                pm = jnp.exp2(sm - m)
                pvv = jnp.exp2(sv - m)
                l = jnp.sum(pm, axis=0, keepdims=True) + jnp.sum(pvv, axis=0, keepdims=True)
                parts = []
                for c in range(NC):
                    for b in range(BPC[c]):
                        j = MSTART[c] + BPC[c] - 1 - b
                        parts.append(pm[j * 16:(j + 1) * 16])
                    if RV[c]:
                        parts.append(pvv[VSTART[c]:VSTART[c] + RV[c]])
                pn = jnp.concatenate(parts, axis=0).astype(bf16)
                a = jnp.dot(vt_scr[h], pn, preferred_element_type=f32)
                ot_scr[qb, pl.ds(pl.multiple_of(h * DH, DH), DH), :] = (a * (1.0 / l)).astype(bf16)
                return carry
            lax.fori_loop(0, H * NQ, body, 0)

    @pl.when(step >= NAS)
    def _():
        fb = step - NAS
        sub = BQ // FSUB
        rng = range(FSUB)
        o = [ot_scr[fb, :, pl.ds(j * sub, sub)].astype(f32).T.astype(bf16) for j in rng]
        h1 = [x_v[pl.ds(pl.multiple_of(fb * BQ + j * sub, sub), sub), :].astype(f32)
              + jnp.dot(o[j], wo_v[...], preferred_element_type=f32) for j in rng]
        hn = [_ln(h1[j]).astype(bf16) for j in rng]
        act = []
        for j in rng:
            gate = lax.dot_general(hn[j], w1t_v[...], NT, preferred_element_type=f32)
            up = lax.dot_general(hn[j], w3t_v[...], NT, preferred_element_type=f32)
            act.append((gate * jax.nn.sigmoid(gate) * up).astype(bf16))
        for j in rng:
            out = h1[j] + jnp.dot(act[j], w2_v[...], preferred_element_type=f32)
            o_ref[pl.ds(j * sub, sub), :] = out.astype(o_ref.dtype)


@jax.jit
def pallas_sequential_preLN__softmax_full_mha__glu_gated_swiglu__prompt_kernel(
    A_x: jax.Array,
    A_wqkv: jax.Array,
    A_wo: jax.Array,
    B_x: jax.Array,
    B_w1: jax.Array,
    B_w3: jax.Array,
    B_w2: jax.Array,
):
    hbm = pl.BlockSpec(memory_space=pl.ANY)
    out = pl.pallas_call(
        _kernel,
        grid=(NAS + NQ,),
        in_specs=[hbm] * 6,
        out_specs=pl.BlockSpec((BQ, D), lambda i: (jnp.maximum(i - NAS, 0), 0)),
        out_shape=jax.ShapeDtypeStruct((S, D), bf16),
        scratch_shapes=[
            pltpu.VMEM((S, D), bf16),
            pltpu.VMEM((D, 3 * D), bf16),
            pltpu.VMEM((D, D), bf16),
            pltpu.VMEM((F, D), bf16),
            pltpu.VMEM((F, D), bf16),
            pltpu.VMEM((F, D), bf16),
            pltpu.VMEM((4, NBP * 16, 128), bf16),
            pltpu.VMEM((4, NV, 128), f32),
            pltpu.VMEM((NQ, D, BQ), bf16),
            pltpu.VMEM((H, DH, S), bf16),
            pltpu.VMEM((NQ, D, BQ), bf16),
            pltpu.VMEM((8, BQ), f32),
            pltpu.VMEM((DH, NV, 128), f32),
            pltpu.VMEM((DH, NV, 128), f32),
            pltpu.VMEM((DH, 8, BQ), f32),
            pltpu.VMEM((DH, 8, BQ), f32),
            pltpu.SemaphoreType.DMA((NQ + 3 + 4,)),
        ],
        compiler_params=pltpu.CompilerParams(dimension_semantics=("arbitrary",),
                                             vmem_limit_bytes=100 * 1024 * 1024),
    )(A_x.reshape(S, D), A_wqkv, A_wo, B_w1.T, B_w3.T, B_w2)
    return out.reshape(1, S, D)
```

```python
import jax
import jax.numpy as jnp
from jax import lax
from jax.experimental import pallas as pl
from jax.experimental.pallas import tpu as pltpu

S, D, H, DH, F = 2048, 512, 32, 16, 1376
LOG2E = 1.4426950408889634
EPS = 1e-5
f32, bf16, u32 = jnp.float32, jnp.bfloat16, jnp.uint32

BQ = 512
NQ = S // BQ
NLT = BQ // 128
C = 128
NC = S // C
HPS = 2
NAS = H // HPS
OFFB = 3
VAHEAD = 5
VPAT = (16, 16, 0)
FSUB = 4
SUB = BQ // FSUB
L_LO, L_HI, A_HI = 2.0 ** -40, 2.0 ** 60, 2.0 ** 100
NT = (((1,), (1,)), ((), ()))

RV = [VPAT[c % len(VPAT)] for c in range(NC)]
RM = [C - v for v in RV]
BPC = [r // 16 for r in RM]
MSTART = [sum(BPC[:c]) for c in range(NC + 1)]
VSTART = [sum(RV[:c]) for c in range(NC + 1)]
NB = MSTART[-1]
NBP = -(-NB // 4) * 4
NV = VSTART[-1]


def _ln(x):
    m = jnp.mean(x, axis=-1, keepdims=True)
    xc = x - m
    v = jnp.mean(xc * xc, axis=-1, keepdims=True)
    return xc * lax.rsqrt(v + EPS)


def _normalise(a, l8):
    l = jnp.sum(l8, axis=0, keepdims=True)
    ok_l = jnp.logical_and(l >= L_LO, l <= L_HI)
    bad_a = jnp.where(jnp.abs(a) <= A_HI, 0.0, 1.0)
    bad = jnp.maximum(jnp.maximum(bad_a[0:8], bad_a[8:16]), jnp.where(ok_l, 0.0, 1.0))
    return (a * (1.0 / l)).astype(bf16), bad


def _kernel(x_hbm, wqkv_hbm, wo_hbm, w1t_hbm, w3t_hbm, w2_hbm, o_hbm,
            x_v, wqkv_v, wo_v, w1t_v, w3t_v, w2_v, out_v,
            k_scr, kv_scr, qt_scr, vt_scr, ot_scr, bad_scr, kb_a, kb_b, p_def, acc_def, l_def,
            sems, osems):
    step = pl.program_id(0)

    def x_copy(i):
        return pltpu.make_async_copy(x_hbm.at[pl.ds(i * BQ, BQ), :], x_v.at[pl.ds(i * BQ, BQ), :], sems.at[i])

    def w_copy(j):
        return pltpu.make_async_copy(wqkv_hbm.at[:, pl.ds(j * D, D)], wqkv_v.at[:, pl.ds(j * D, D)], sems.at[NQ + j])

    late = [(wo_hbm, wo_v), (w1t_hbm, w1t_v), (w3t_hbm, w3t_v), (w2_hbm, w2_v)]

    def late_copy(j):
        return pltpu.make_async_copy(late[j][0], late[j][1], sems.at[NQ + 3 + j])

    def out_copy(r0, i):
        return pltpu.make_async_copy(out_v.at[pl.ds(r0, SUB), :], o_hbm.at[pl.ds(r0, SUB), :], osems.at[i])

    def k_rows(g, blk0, nblk):
        return pltpu.bitcast(k_scr[g, pl.ds(blk0 * 8, nblk * 8), :], bf16)

    def masked_qt(h, qb):
        qt = qt_scr[qb, pl.ds(pl.multiple_of((h // 8) * 128, 128), 128), :]
        rows = lax.broadcasted_iota(jnp.int32, (128, BQ), 0) // DH
        return jnp.where(rows == h % 8, qt.astype(f32), 0.0).astype(bf16)

    def produce_kb(h, kb):
        x = pltpu.roll(kv_scr[h // 8], (128 - (h % 8) * DH) % 128, 1)
        for d in range(DH):
            kb[d] = jnp.broadcast_to(x[:, d:d + 1], (NV, 128))

    def deferred_pv(h):
        a = acc_def[...] + jnp.dot(vt_scr[h, :, pl.ds((NC - 1) * C, C)], pltpu.bitcast(p_def[...], bf16),
                                   preferred_element_type=f32)
        o, bad = _normalise(a, l_def[...])
        ot_scr[NQ - 1, pl.ds(pl.multiple_of(h * DH, DH), DH), :] = o
        return bad

    @pl.when(step == 0)
    def _():
        x_copy(0).start()
        w_copy(1).start()
        w_copy(0).start()
        w_copy(2).start()
        for i in range(1, NQ):
            x_copy(i).start()
        bad_scr[...] = jnp.zeros_like(bad_scr)
        p_def[...] = jnp.zeros_like(p_def)
        acc_def[...] = jnp.zeros_like(acc_def)
        l_def[...] = jnp.ones_like(l_def)

        def proj_k(qb, xn):
            k = jnp.dot(xn, wqkv_v[:, D:2 * D], preferred_element_type=f32).astype(bf16)
            for cc in range(BQ // C):
                c = qb * (BQ // C) + cc
                for b in range(BPC[c]):
                    r0 = cc * C + (BPC[c] - 1 - b) * 16
                    for g in range(4):
                        k_scr[g, pl.ds((MSTART[c] + b) * 8, 8), :] = pltpu.bitcast(
                            k[r0:r0 + 16, g * 128:(g + 1) * 128], u32)
                if RV[c]:
                    r0 = cc * C + RM[c]
                    kf = k[r0:r0 + RV[c]].astype(f32)
                    for g in range(4):
                        kv_scr[g, pl.ds(VSTART[c], RV[c]), :] = kf[:, g * 128:(g + 1) * 128]

        def proj_q(qb, xn, wq_t):
            qt = lax.dot_general(wq_t, xn, NT, preferred_element_type=f32)
            qt_scr[qb] = (qt * (DH ** -0.5 * LOG2E)).astype(bf16)

        def proj_v(qb, xn, wv_t):
            vt = lax.dot_general(wv_t, xn, NT, preferred_element_type=f32)
            vt_scr[:, :, pl.ds(qb * BQ, BQ)] = vt.astype(bf16).reshape(H, DH, BQ)

        def ln_chunk(qb):
            return _ln(x_v[pl.ds(qb * BQ, BQ), :].astype(f32)).astype(bf16)

        x_copy(0).wait()
        xn0 = ln_chunk(0)
        w_copy(1).wait()
        proj_k(0, xn0)
        w_copy(0).wait()
        wq_t = wqkv_v[:, 0:D].astype(f32).T.astype(bf16)
        proj_q(0, xn0, wq_t)
        for j in range(len(late)):
            late_copy(j).start()
        w_copy(2).wait()
        x_copy(1).wait()
        wv_t = wqkv_v[:, 2 * D:3 * D].astype(f32).T.astype(bf16)
        xn1 = ln_chunk(1)
        proj_v(0, xn0, wv_t)
        for i in range(2, NQ):
            x_copy(i).wait()
        for qb in range(1, NQ):
            xn = xn1 if qb == 1 else ln_chunk(qb)
            proj_k(qb, xn)
            proj_q(qb, xn, wq_t)
            proj_v(qb, xn, wv_t)
        produce_kb(0, kb_a)

    @pl.when(step < NAS)
    def _():
        h0 = step * HPS
        items = [(u, qb) for u in range(HPS) for qb in range(NQ)]
        kbs = [kb_a, kb_b]
        qms, qbv, blk, acc, lacc, vout = {}, {}, {}, {}, {}, {}
        chunks = [(it, c) for it in range(len(items)) for c in range(NC)]
        vpieces = [(it, c, lt, hf) for (it, c) in chunks if RV[c] for lt in range(NLT) for hf in range(2)]
        st = {"bad": None, "link": None, "vi": 0, "cur": None}

        def add_bad(b):
            st["bad"] = b if st["bad"] is None else jnp.maximum(st["bad"], b)

        def emit_vpiece():
            if st["vi"] >= len(vpieces):
                return
            it, c, lt, hf = vpieces[st["vi"]]
            st["vi"] += 1
            u, qb = items[it]
            if it not in qbv:
                q16 = qt_scr[qb, pl.ds(pl.multiple_of((h0 + u) * DH, DH), DH), :].astype(f32)
                qbv[it] = [jnp.broadcast_to(q16[d:d + 1, :], (8, BQ)) for d in range(DH)]
            if hf == 0:
                a = None if st["link"] is None else st["link"] - st["link"]
            else:
                a = st["cur"]
            for d in range(hf * 8, hf * 8 + 8):
                kbd = kbs[u % 2][d, pl.ds(VSTART[c], RV[c]), :]
                qbb = jnp.concatenate([qbv[it][d][:, lt * 128:(lt + 1) * 128]] * (RV[c] // 8), axis=0)
                term = kbd * qbb
                a = term if a is None else a + term
            st["cur"] = a
            if hf == 1:
                vout.setdefault((it, c), []).append(a)
                st["link"] = a

        def sum_add(it, p16, j):
            s2 = p16[0:8] + p16[8:16]
            key = (it, j % 2)
            lacc[key] = s2 if key not in lacc else lacc[key] + s2

        def emit_pv(ci):
            it, c = chunks[ci]
            u, qb = items[it]
            if c == 1 and qb == 0:
                produce_kb(jnp.minimum(h0 + u + 1, H - 1), kbs[(u + 1) % 2])
            while RV[c] and len(vout.get((it, c), [])) < NLT:
                emit_vpiece()
            target = len([cc for cc in chunks[:ci + 1 + VAHEAD] if RV[cc[1]]]) * NLT * 2
            todo = max(target - st["vi"], 0)
            ps = []
            if RV[c]:
                pvv = jnp.exp2(jnp.concatenate(vout.pop((it, c)), axis=1))
                sum_add(it, pvv, 0)
            for b in range(BPC[c]):
                p16 = jnp.exp2(blk.pop((it, MSTART[c] + b)))
                sum_add(it, p16, b + 1)
                ps.append(p16)
                for _ in range((todo * (b + 1)) // BPC[c] - (todo * b) // BPC[c]):
                    emit_vpiece()
            ps = ps[::-1]
            if RV[c]:
                ps.append(pvv)
            p = jnp.concatenate(ps, axis=0).astype(bf16)
            if ci == len(chunks) - 1:
                p_def[...] = pltpu.bitcast(p, u32)
                acc_def[...] = acc.pop(it)
                l_def[...] = lacc.pop((it, 0)) + lacc.pop((it, 1))
                return
            pv = jnp.dot(vt_scr[h0 + u, :, pl.ds(c * C, C)], p, preferred_element_type=f32)
            acc[it] = pv if c == 0 else acc[it] + pv
            if c == NC - 1:
                o, bad = _normalise(acc.pop(it), lacc.pop((it, 0)) + lacc.pop((it, 1)))
                add_bad(bad)
                ot_scr[qb, pl.ds(pl.multiple_of((h0 + u) * DH, DH), DH), :] = o

        add_bad(deferred_pv(jnp.maximum(h0 - 1, 0)))
        pvi = 0
        for it, (u, qb) in enumerate(items):
            qms[it] = masked_qt(h0 + u, qb)
            bounds = sorted(set([0, NB] + [MSTART[c] + OFFB for c in range(NC) if MSTART[c] + OFFB < NB]))
            for a, b in zip(bounds[:-1], bounds[1:]):
                sm = jnp.dot(k_rows((h0 + u) // 8, a, b - a), qms[it], preferred_element_type=f32)
                for j in range(a, b):
                    blk[(it, j)] = sm[(j - a) * 16:(j - a + 1) * 16]
                pos = it * NB + b
                while pvi < len(chunks):
                    cit, cc = chunks[pvi]
                    nxt = cc + 2
                    need = cit * NB + MSTART[nxt] if nxt <= NC else (cit + 1) * NB + MSTART[nxt - NC]
                    if need + OFFB > pos:
                        break
                    emit_pv(pvi)
                    pvi += 1
        while pvi < len(chunks):
            emit_pv(pvi)
            pvi += 1
        bad_scr[...] = jnp.maximum(bad_scr[...], st["bad"])

    @pl.when(step == NAS)
    def _():
        for j in range(len(late)):
            late_copy(j).wait()
        bad = jnp.maximum(bad_scr[...], deferred_pv(H - 1))

        @pl.when(jnp.max(bad) > 0.0)
        def _():
            def body(i, carry):
                h = i // NQ
                qb = i % NQ
                qm = masked_qt(h, qb)
                sm = jnp.dot(k_rows(h // 8, 0, NB), qm, preferred_element_type=f32)
                sv = jnp.dot(kv_scr[h // 8].astype(bf16), qm, preferred_element_type=f32)
                m = jnp.maximum(jnp.max(sm, axis=0, keepdims=True), jnp.max(sv, axis=0, keepdims=True))
                pm = jnp.exp2(sm - m)
                pvv = jnp.exp2(sv - m)
                l = jnp.sum(pm, axis=0, keepdims=True) + jnp.sum(pvv, axis=0, keepdims=True)
                parts = []
                for c in range(NC):
                    for b in range(BPC[c]):
                        j = MSTART[c] + BPC[c] - 1 - b
                        parts.append(pm[j * 16:(j + 1) * 16])
                    if RV[c]:
                        parts.append(pvv[VSTART[c]:VSTART[c] + RV[c]])
                pn = jnp.concatenate(parts, axis=0).astype(bf16)
                a = jnp.dot(vt_scr[h], pn, preferred_element_type=f32)
                ot_scr[qb, pl.ds(pl.multiple_of(h * DH, DH), DH), :] = (a * (1.0 / l)).astype(bf16)
                return carry
            lax.fori_loop(0, H * NQ, body, 0)

    @pl.when(step >= NAS)
    def _():
        fb = step - NAS
        rng = range(FSUB)
        r0 = [pl.multiple_of(fb * BQ + j * SUB, SUB) for j in rng]
        o = [ot_scr[fb, :, pl.ds(j * SUB, SUB)].astype(f32).T.astype(bf16) for j in rng]
        h1 = [x_v[pl.ds(r0[j], SUB), :].astype(f32) + jnp.dot(o[j], wo_v[...], preferred_element_type=f32)
              for j in rng]
        hn = [_ln(h1[j]).astype(bf16) for j in rng]
        act = []
        for j in rng:
            gate = lax.dot_general(hn[j], w1t_v[...], NT, preferred_element_type=f32)
            up = lax.dot_general(hn[j], w3t_v[...], NT, preferred_element_type=f32)
            act.append((gate * jax.nn.sigmoid(gate) * up).astype(bf16))
        for j in rng:
            out = h1[j] + jnp.dot(act[j], w2_v[...], preferred_element_type=f32)
            out_v[pl.ds(r0[j], SUB), :] = out.astype(bf16)
            out_copy(r0[j], fb * FSUB + j).start()

    @pl.when(step == NAS + NQ - 1)
    def _():
        for i in range(NQ * FSUB):
            out_copy(i * SUB, i).wait()


@jax.jit
def pallas_sequential_preLN__softmax_full_mha__glu_gated_swiglu__prompt_kernel(
    A_x: jax.Array,
    A_wqkv: jax.Array,
    A_wo: jax.Array,
    B_x: jax.Array,
    B_w1: jax.Array,
    B_w3: jax.Array,
    B_w2: jax.Array,
):
    hbm = pl.BlockSpec(memory_space=pl.ANY)
    out = pl.pallas_call(
        _kernel,
        grid=(NAS + NQ,),
        in_specs=[hbm] * 6,
        out_specs=hbm,
        out_shape=jax.ShapeDtypeStruct((S, D), bf16),
        scratch_shapes=[
            pltpu.VMEM((S, D), bf16),
            pltpu.VMEM((D, 3 * D), bf16),
            pltpu.VMEM((D, D), bf16),
            pltpu.VMEM((F, D), bf16),
            pltpu.VMEM((F, D), bf16),
            pltpu.VMEM((F, D), bf16),
            pltpu.VMEM((S, D), bf16),
            pltpu.VMEM((4, NBP * 8, 128), u32),
            pltpu.VMEM((4, NV, 128), f32),
            pltpu.VMEM((NQ, D, BQ), bf16),
            pltpu.VMEM((H, DH, S), bf16),
            pltpu.VMEM((NQ, D, BQ), bf16),
            pltpu.VMEM((8, BQ), f32),
            pltpu.VMEM((DH, NV, 128), f32),
            pltpu.VMEM((DH, NV, 128), f32),
            pltpu.VMEM((C // 2, BQ), u32),
            pltpu.VMEM((DH, BQ), f32),
            pltpu.VMEM((8, BQ), f32),
            pltpu.SemaphoreType.DMA((NQ + 3 + 4,)),
            pltpu.SemaphoreType.DMA((NQ * FSUB,)),
        ],
        compiler_params=pltpu.CompilerParams(dimension_semantics=("arbitrary",),
                                             vmem_limit_bytes=100 * 1024 * 1024),
    )(A_x.reshape(S, D), A_wqkv, A_wo, B_w1.T, B_w3.T, B_w2)
    return out.reshape(1, S, D)
```

```python
import jax
import jax.numpy as jnp
from jax import lax
from jax.experimental import pallas as pl
from jax.experimental.pallas import tpu as pltpu

S, D, H, DH, F = 2048, 512, 32, 16, 1376
LOG2E = 1.4426950408889634
EPS = 1e-5
f32, bf16, u32 = jnp.float32, jnp.bfloat16, jnp.uint32

BQ = 512
NQ = S // BQ
NLT = BQ // 128
C = 128
NC = S // C
HPS = 2
NAS = H // HPS
OFFB = 3
VAHEAD = 5
VPAT = (16,) * 15 + (0,)
NTH = 2
TOKP = "rr-"
FSUB = 4
SUB = BQ // FSUB
L_LO, L_HI, A_HI = 2.0 ** -40, 2.0 ** 60, 2.0 ** 100
NT = (((1,), (1,)), ((), ()))

RV = [VPAT[c % len(VPAT)] for c in range(NC)]
RM = [C - v for v in RV]
BPC = [r // 16 for r in RM]
MSTART = [sum(BPC[:c]) for c in range(NC + 1)]
VSTART = [sum(RV[:c]) for c in range(NC + 1)]
NB = MSTART[-1]
NBP = -(-NB // 4) * 4
NV = VSTART[-1]


def _ln(x):
    m = jnp.mean(x, axis=-1, keepdims=True)
    xc = x - m
    v = jnp.mean(xc * xc, axis=-1, keepdims=True)
    return xc * lax.rsqrt(v + EPS)


def _normalise(a, l8):
    l = jnp.sum(l8, axis=0, keepdims=True)
    ok_l = jnp.logical_and(l >= L_LO, l <= L_HI)
    bad_a = jnp.where(jnp.abs(a) <= A_HI, 0.0, 1.0)
    bad = jnp.maximum(jnp.maximum(bad_a[0:8], bad_a[8:16]), jnp.where(ok_l, 0.0, 1.0))
    return (a * (1.0 / l)).astype(bf16), bad


def _kernel(x_hbm, wqkv_hbm, wo_hbm, w1t_hbm, w3t_hbm, w2_hbm, o_hbm,
            x_v, wqkv_v, wo_v, w1t_v, w3t_v, w2_v, out_v,
            k_scr, kv_scr, qt_scr, vt_scr, ot_scr, bad_scr, kb_a, kb_b, p_def, acc_def, l_def,
            sems, osems):
    step = pl.program_id(0)

    def x_copy(i):
        return pltpu.make_async_copy(x_hbm.at[pl.ds(i * BQ, BQ), :], x_v.at[pl.ds(i * BQ, BQ), :], sems.at[i])

    def w_copy(j):
        return pltpu.make_async_copy(wqkv_hbm.at[:, pl.ds(j * D, D)], wqkv_v.at[:, pl.ds(j * D, D)], sems.at[NQ + j])

    late = [(wo_hbm, wo_v), (w1t_hbm, w1t_v), (w3t_hbm, w3t_v), (w2_hbm, w2_v)]

    def late_copy(j):
        return pltpu.make_async_copy(late[j][0], late[j][1], sems.at[NQ + 3 + j])

    def out_copy(r0, i):
        return pltpu.make_async_copy(out_v.at[pl.ds(r0, SUB), :], o_hbm.at[pl.ds(r0, SUB), :], osems.at[i])

    def k_rows(g, blk0, nblk):
        return pltpu.bitcast(k_scr[g, pl.ds(blk0 * 8, nblk * 8), :], bf16)

    def masked_qt(h, qb):
        qt = qt_scr[qb, pl.ds(pl.multiple_of((h // 8) * 128, 128), 128), :]
        rows = lax.broadcasted_iota(jnp.int32, (128, BQ), 0) // DH
        return jnp.where(rows == h % 8, qt.astype(f32), 0.0).astype(bf16)

    def produce_kb(h, kb):
        x = pltpu.roll(kv_scr[h // 8], (128 - (h % 8) * DH) % 128, 1)
        for d in range(DH):
            kb[d] = jnp.broadcast_to(x[:, d:d + 1], (NV, 128))

    def deferred_pv(h):
        a = acc_def[...] + jnp.dot(vt_scr[h, :, pl.ds((NC - 1) * C, C)], p_def[...], preferred_element_type=f32)
        o, bad = _normalise(a, l_def[...])
        ot_scr[NQ - 1, pl.ds(pl.multiple_of(h * DH, DH), DH), :] = o
        return bad

    @pl.when(step == 0)
    def _():
        x_copy(0).start()
        w_copy(1).start()
        w_copy(0).start()
        w_copy(2).start()
        for i in range(1, NQ):
            x_copy(i).start()
        bad_scr[...] = jnp.zeros_like(bad_scr)
        p_def[...] = jnp.zeros_like(p_def)
        acc_def[...] = jnp.zeros_like(acc_def)
        l_def[...] = jnp.ones_like(l_def)

        def proj_k(qb, xn):
            k = jnp.dot(xn, wqkv_v[:, D:2 * D], preferred_element_type=f32).astype(bf16)
            for cc in range(BQ // C):
                c = qb * (BQ // C) + cc
                for b in range(BPC[c]):
                    r0 = cc * C + (BPC[c] - 1 - b) * 16
                    for g in range(4):
                        k_scr[g, pl.ds((MSTART[c] + b) * 8, 8), :] = pltpu.bitcast(
                            k[r0:r0 + 16, g * 128:(g + 1) * 128], u32)
                if RV[c]:
                    r0 = cc * C + RM[c]
                    kf = k[r0:r0 + RV[c]].astype(f32)
                    for g in range(4):
                        kv_scr[g, pl.ds(VSTART[c], RV[c]), :] = kf[:, g * 128:(g + 1) * 128]

        def proj_q(qb, xn, wq_t):
            qt = lax.dot_general(wq_t, xn, NT, preferred_element_type=f32)
            qt_scr[qb] = (qt * (DH ** -0.5 * LOG2E)).astype(bf16)

        def proj_v(qb, xn, wv_t):
            vt = lax.dot_general(wv_t, xn, NT, preferred_element_type=f32)
            vt_scr[:, :, pl.ds(qb * BQ, BQ)] = vt.astype(bf16).astype(f32).reshape(H, DH, BQ)

        def ln_chunk(qb):
            return _ln(x_v[pl.ds(qb * BQ, BQ), :].astype(f32)).astype(bf16)

        x_copy(0).wait()
        xn0 = ln_chunk(0)
        w_copy(1).wait()
        proj_k(0, xn0)
        w_copy(0).wait()
        wq_t = wqkv_v[:, 0:D].astype(f32).T.astype(bf16)
        proj_q(0, xn0, wq_t)
        for j in range(len(late)):
            late_copy(j).start()
        w_copy(2).wait()
        x_copy(1).wait()
        wv_t = wqkv_v[:, 2 * D:3 * D].astype(f32).T.astype(bf16)
        xn1 = ln_chunk(1)
        proj_v(0, xn0, wv_t)
        for i in range(2, NQ):
            x_copy(i).wait()
        for qb in range(1, NQ):
            xn = xn1 if qb == 1 else ln_chunk(qb)
            proj_k(qb, xn)
            proj_q(qb, xn, wq_t)
            proj_v(qb, xn, wv_t)
        produce_kb(0, kb_a)

    @pl.when(step < NAS)
    def _():
        h0 = step * HPS
        items = [(u, qb) for u in range(HPS) for qb in range(NQ)]
        kbs = [kb_a, kb_b]
        qms, qbv, blk, acc, lacc, vout = {}, {}, {}, {}, {}, {}
        chunks = [(it, c) for it in range(len(items)) for c in range(NC)]
        vpieces = [(it, c, lt, hf) for (it, c) in chunks if RV[c] for lt in range(NLT) for hf in range(2)]
        st = {"bad": None, "vi": 0, "cur": None, "tok": None}
        links = {}

        def add_bad(b):
            st["bad"] = b if st["bad"] is None else jnp.maximum(st["bad"], b)

        def emit_vpiece():
            if st["vi"] >= len(vpieces):
                return
            it, c, lt, hf = vpieces[st["vi"]]
            st["vi"] += 1
            u, qb = items[it]
            if it not in qbv:
                q16 = qt_scr[qb, pl.ds(pl.multiple_of((h0 + u) * DH, DH), DH), :].astype(f32)
                qbv[it] = [jnp.broadcast_to(q16[d:d + 1, :], (8, BQ)) for d in range(DH)]
            if hf == 0:
                lk = links.get(lt % NTH)
                a = None if lk is None else lk - lk
            else:
                a = st["cur"]
            for d in range(hf * 8, hf * 8 + 8):
                kbd = kbs[u % 2][d, pl.ds(VSTART[c], RV[c]), :]
                qbb = jnp.concatenate([qbv[it][d][:, lt * 128:(lt + 1) * 128]] * (RV[c] // 8), axis=0)
                term = kbd * qbb
                a = term if a is None else a + term
            st["cur"] = a
            if hf == 1:
                vout.setdefault((it, c), []).append(a)
                links[lt % NTH] = a

        def sum_add(it, p16, j):
            s2 = p16[0:8] + p16[8:16]
            key = (it, j % 2)
            lacc[key] = s2 if key not in lacc else lacc[key] + s2

        def emit_pv(ci):
            it, c = chunks[ci]
            u, qb = items[it]
            if c == 1 and qb == 0:
                produce_kb(jnp.minimum(h0 + u + 1, H - 1), kbs[(u + 1) % 2])
            while RV[c] and len(vout.get((it, c), [])) < NLT:
                emit_vpiece()
            target = len([cc for cc in chunks[:ci + 1 + VAHEAD] if RV[cc[1]]]) * NLT * 2
            todo = max(target - st["vi"], 0)
            ps = []
            if RV[c]:
                pvv = jnp.exp2(jnp.concatenate(vout.pop((it, c)), axis=1))
                sum_add(it, pvv, 0)
            for b in range(BPC[c]):
                p16 = jnp.exp2(blk.pop((it, MSTART[c] + b)))
                sum_add(it, p16, b + 1)
                ps.append(p16)
                for _ in range((todo * (b + 1)) // BPC[c] - (todo * b) // BPC[c]):
                    emit_vpiece()
            ps = ps[::-1]
            if RV[c]:
                ps.append(pvv)
            p = jnp.concatenate(ps, axis=0)
            if ci == len(chunks) - 1:
                p_def[...] = p
                acc_def[...] = acc.pop(it)
                l_def[...] = lacc.pop((it, 0)) + lacc.pop((it, 1))
                return
            pv = jnp.dot(vt_scr[h0 + u, :, pl.ds(c * C, C)], p, preferred_element_type=f32)
            z = pv[0:8, 0:128] - pv[0:8, 0:128]
            t = z if st["tok"] is None else st["tok"] + z
            st["tok"] = pltpu.roll(t, 1, 1) if TOKP[ci % len(TOKP)] == "r" else t
            acc[it] = pv if c == 0 else acc[it] + pv
            if c == NC - 1:
                o, bad = _normalise(acc.pop(it), lacc.pop((it, 0)) + lacc.pop((it, 1)))
                add_bad(bad)
                ot_scr[qb, pl.ds(pl.multiple_of((h0 + u) * DH, DH), DH), :] = o

        add_bad(deferred_pv(jnp.maximum(h0 - 1, 0)))
        pvi = 0
        for it, (u, qb) in enumerate(items):
            qms[it] = masked_qt(h0 + u, qb)
            bounds = sorted(set([0, NB] + [MSTART[c] + OFFB for c in range(NC) if MSTART[c] + OFFB < NB]))
            for a, b in zip(bounds[:-1], bounds[1:]):
                sm = jnp.dot(k_rows((h0 + u) // 8, a, b - a), qms[it], preferred_element_type=f32)
                for j in range(a, b):
                    blk[(it, j)] = sm[(j - a) * 16:(j - a + 1) * 16]
                pos = it * NB + b
                while pvi < len(chunks):
                    cit, cc = chunks[pvi]
                    nxt = cc + 2
                    need = cit * NB + MSTART[nxt] if nxt <= NC else (cit + 1) * NB + MSTART[nxt - NC]
                    if need + OFFB > pos:
                        break
                    emit_pv(pvi)
                    pvi += 1
        while pvi < len(chunks):
            emit_pv(pvi)
            pvi += 1
        tok_bad = jnp.where(st["tok"] == 0.0, 0.0, 1.0)
        add_bad(jnp.concatenate([tok_bad] * NLT, axis=1))
        bad_scr[...] = jnp.maximum(bad_scr[...], st["bad"])

    @pl.when(step == NAS)
    def _():
        for j in range(len(late)):
            late_copy(j).wait()
        bad = jnp.maximum(bad_scr[...], deferred_pv(H - 1))

        @pl.when(jnp.max(bad) > 0.0)
        def _():
            def body(i, carry):
                h = i // NQ
                qb = i % NQ
                qm = masked_qt(h, qb)
                sm = jnp.dot(k_rows(h // 8, 0, NB), qm, preferred_element_type=f32)
                sv = jnp.dot(kv_scr[h // 8].astype(bf16), qm, preferred_element_type=f32)
                m = jnp.maximum(jnp.max(sm, axis=0, keepdims=True), jnp.max(sv, axis=0, keepdims=True))
                pm = jnp.exp2(sm - m)
                pvv = jnp.exp2(sv - m)
                l = jnp.sum(pm, axis=0, keepdims=True) + jnp.sum(pvv, axis=0, keepdims=True)
                parts = []
                for c in range(NC):
                    for b in range(BPC[c]):
                        j = MSTART[c] + BPC[c] - 1 - b
                        parts.append(pm[j * 16:(j + 1) * 16])
                    if RV[c]:
                        parts.append(pvv[VSTART[c]:VSTART[c] + RV[c]])
                pn = jnp.concatenate(parts, axis=0)
                a = jnp.dot(vt_scr[h], pn, preferred_element_type=f32)
                ot_scr[qb, pl.ds(pl.multiple_of(h * DH, DH), DH), :] = (a * (1.0 / l)).astype(bf16)
                return carry
            lax.fori_loop(0, H * NQ, body, 0)

    @pl.when(step >= NAS)
    def _():
        fb = step - NAS
        rng = range(FSUB)
        r0 = [pl.multiple_of(fb * BQ + j * SUB, SUB) for j in rng]
        o = [ot_scr[fb, :, pl.ds(j * SUB, SUB)].astype(f32).T.astype(bf16) for j in rng]
        h1 = [x_v[pl.ds(r0[j], SUB), :].astype(f32) + jnp.dot(o[j], wo_v[...], preferred_element_type=f32)
              for j in rng]
        hn = [_ln(h1[j]).astype(bf16) for j in rng]
        act = []
        for j in rng:
            gate = lax.dot_general(hn[j], w1t_v[...], NT, preferred_element_type=f32)
            up = lax.dot_general(hn[j], w3t_v[...], NT, preferred_element_type=f32)
            act.append((gate * jax.nn.sigmoid(gate) * up).astype(bf16))
        for j in rng:
            out = h1[j] + jnp.dot(act[j], w2_v[...], preferred_element_type=f32)
            out_v[pl.ds(r0[j], SUB), :] = out.astype(bf16)
            out_copy(r0[j], fb * FSUB + j).start()

    @pl.when(step == NAS + NQ - 1)
    def _():
        for i in range(NQ * FSUB):
            out_copy(i * SUB, i).wait()


@jax.jit
def pallas_sequential_preLN__softmax_full_mha__glu_gated_swiglu__prompt_kernel(
    A_x: jax.Array,
    A_wqkv: jax.Array,
    A_wo: jax.Array,
    B_x: jax.Array,
    B_w1: jax.Array,
    B_w3: jax.Array,
    B_w2: jax.Array,
):
    hbm = pl.BlockSpec(memory_space=pl.ANY)
    out = pl.pallas_call(
        _kernel,
        grid=(NAS + NQ,),
        in_specs=[hbm] * 6,
        out_specs=hbm,
        out_shape=jax.ShapeDtypeStruct((S, D), bf16),
        scratch_shapes=[
            pltpu.VMEM((S, D), bf16),
            pltpu.VMEM((D, 3 * D), bf16),
            pltpu.VMEM((D, D), bf16),
            pltpu.VMEM((F, D), bf16),
            pltpu.VMEM((F, D), bf16),
            pltpu.VMEM((F, D), bf16),
            pltpu.VMEM((S, D), bf16),
            pltpu.VMEM((4, NBP * 8, 128), u32),
            pltpu.VMEM((4, NV, 128), f32),
            pltpu.VMEM((NQ, D, BQ), bf16),
            pltpu.VMEM((H, DH, S), f32),
            pltpu.VMEM((NQ, D, BQ), bf16),
            pltpu.VMEM((8, BQ), f32),
            pltpu.VMEM((DH, NV, 128), f32),
            pltpu.VMEM((DH, NV, 128), f32),
            pltpu.VMEM((C, BQ), f32),
            pltpu.VMEM((DH, BQ), f32),
            pltpu.VMEM((8, BQ), f32),
            pltpu.SemaphoreType.DMA((NQ + 3 + 4,)),
            pltpu.SemaphoreType.DMA((NQ * FSUB,)),
        ],
        compiler_params=pltpu.CompilerParams(dimension_semantics=("arbitrary",),
                                             vmem_limit_bytes=100 * 1024 * 1024),
    )(A_x.reshape(S, D), A_wqkv, A_wo, B_w1.T, B_w3.T, B_w2)
    return out.reshape(1, S, D)
```

```python
import jax
import jax.numpy as jnp
from jax import lax
from jax.experimental import pallas as pl
from jax.experimental.pallas import tpu as pltpu

S, D, H, DH, F = 2048, 512, 32, 16, 1376
LOG2E = 1.4426950408889634
EPS = 1e-5
f32, bf16, u32 = jnp.float32, jnp.bfloat16, jnp.uint32

BQ = 512
NQ = S // BQ
NLT = BQ // 128
C = 128
NC = S // C
HPS = 2
NAS = H // HPS
OFFB = 2
VAHEAD = 5
VPAT = (16,) * 15 + (0,)
NTH = 3
TOKP = "rr-"
FSUB = 4
SUB = BQ // FSUB
L_LO, L_HI, A_HI = 2.0 ** -40, 2.0 ** 60, 2.0 ** 100
NT = (((1,), (1,)), ((), ()))

RV = [VPAT[c % len(VPAT)] for c in range(NC)]
RM = [C - v for v in RV]
BPC = [r // 16 for r in RM]
MSTART = [sum(BPC[:c]) for c in range(NC + 1)]
VSTART = [sum(RV[:c]) for c in range(NC + 1)]
NB = MSTART[-1]
NBP = -(-NB // 4) * 4
NV = VSTART[-1]


def _ln(x):
    m = jnp.mean(x, axis=-1, keepdims=True)
    xc = x - m
    v = jnp.mean(xc * xc, axis=-1, keepdims=True)
    return xc * lax.rsqrt(v + EPS)


def _normalise(a, l8):
    l = jnp.sum(l8, axis=0, keepdims=True)
    ok_l = jnp.logical_and(l >= L_LO, l <= L_HI)
    bad_a = jnp.where(jnp.abs(a) <= A_HI, 0.0, 1.0)
    bad = jnp.maximum(jnp.maximum(bad_a[0:8], bad_a[8:16]), jnp.where(ok_l, 0.0, 1.0))
    return (a * (1.0 / l)).astype(bf16), bad


def _kernel(x_hbm, wqkv_hbm, wo_hbm, w1t_hbm, w3t_hbm, w2_hbm, o_hbm,
            x_v, wqkv_v, wo_v, w1t_v, w3t_v, w2_v, out_v,
            k_scr, kv_scr, qt_scr, vt_scr, ot_scr, bad_scr, kb_a, kb_b, p_def, acc_def, l_def,
            sems, osems):
    step = pl.program_id(0)

    def x_copy(i):
        return pltpu.make_async_copy(x_hbm.at[pl.ds(i * BQ, BQ), :], x_v.at[pl.ds(i * BQ, BQ), :], sems.at[i])

    def w_copy(j):
        return pltpu.make_async_copy(wqkv_hbm.at[:, pl.ds(j * D, D)], wqkv_v.at[:, pl.ds(j * D, D)], sems.at[NQ + j])

    late = [(wo_hbm, wo_v), (w1t_hbm, w1t_v), (w3t_hbm, w3t_v), (w2_hbm, w2_v)]

    def late_copy(j):
        return pltpu.make_async_copy(late[j][0], late[j][1], sems.at[NQ + 3 + j])

    def out_copy(r0, i):
        return pltpu.make_async_copy(out_v.at[pl.ds(r0, SUB), :], o_hbm.at[pl.ds(r0, SUB), :], osems.at[i])

    def k_rows(g, blk0, nblk):
        return pltpu.bitcast(k_scr[g, pl.ds(blk0 * 8, nblk * 8), :], bf16)

    def masked_qt(h, qb):
        qt = qt_scr[qb, pl.ds(pl.multiple_of((h // 8) * 128, 128), 128), :]
        rows = lax.broadcasted_iota(jnp.int32, (128, BQ), 0) // DH
        return jnp.where(rows == h % 8, qt.astype(f32), 0.0).astype(bf16)

    def produce_kb(h, kb):
        x = pltpu.roll(kv_scr[h // 8], (128 - (h % 8) * DH) % 128, 1)
        for d in range(DH):
            kb[d] = jnp.broadcast_to(x[:, d:d + 1], (NV, 128))

    def deferred_pv(h):
        a = acc_def[...] + jnp.dot(vt_scr[h, :, pl.ds((NC - 1) * C, C)], p_def[...], preferred_element_type=f32)
        o, bad = _normalise(a, l_def[...])
        ot_scr[NQ - 1, pl.ds(pl.multiple_of(h * DH, DH), DH), :] = o
        return bad

    @pl.when(step == 0)
    def _():
        x_copy(0).start()
        w_copy(1).start()
        w_copy(0).start()
        w_copy(2).start()
        for i in range(1, NQ):
            x_copy(i).start()
        bad_scr[...] = jnp.zeros_like(bad_scr)
        p_def[...] = jnp.zeros_like(p_def)
        acc_def[...] = jnp.zeros_like(acc_def)
        l_def[...] = jnp.ones_like(l_def)

        def proj_k(qb, xn):
            k = jnp.dot(xn, wqkv_v[:, D:2 * D], preferred_element_type=f32).astype(bf16)
            for cc in range(BQ // C):
                c = qb * (BQ // C) + cc
                for b in range(BPC[c]):
                    r0 = cc * C + (BPC[c] - 1 - b) * 16
                    for g in range(4):
                        k_scr[g, pl.ds((MSTART[c] + b) * 8, 8), :] = pltpu.bitcast(
                            k[r0:r0 + 16, g * 128:(g + 1) * 128], u32)
                if RV[c]:
                    r0 = cc * C + RM[c]
                    kf = k[r0:r0 + RV[c]].astype(f32)
                    for g in range(4):
                        kv_scr[g, pl.ds(VSTART[c], RV[c]), :] = kf[:, g * 128:(g + 1) * 128]

        def proj_q(qb, xn, wq_t):
            qt = lax.dot_general(wq_t, xn, NT, preferred_element_type=f32)
            qt_scr[qb] = (qt * (DH ** -0.5 * LOG2E)).astype(bf16)

        def proj_v(qb, xn, wv_t):
            vt = lax.dot_general(wv_t, xn, NT, preferred_element_type=f32)
            vt_scr[:, :, pl.ds(qb * BQ, BQ)] = vt.astype(bf16).astype(f32).reshape(H, DH, BQ)

        def ln_chunk(qb):
            return _ln(x_v[pl.ds(qb * BQ, BQ), :].astype(f32)).astype(bf16)

        x_copy(0).wait()
        xn0 = ln_chunk(0)
        w_copy(1).wait()
        proj_k(0, xn0)
        w_copy(0).wait()
        wq_t = wqkv_v[:, 0:D].astype(f32).T.astype(bf16)
        proj_q(0, xn0, wq_t)
        for j in range(len(late)):
            late_copy(j).start()
        w_copy(2).wait()
        x_copy(1).wait()
        wv_t = wqkv_v[:, 2 * D:3 * D].astype(f32).T.astype(bf16)
        xn1 = ln_chunk(1)
        proj_v(0, xn0, wv_t)
        for i in range(2, NQ):
            x_copy(i).wait()
        for qb in range(1, NQ):
            xn = xn1 if qb == 1 else ln_chunk(qb)
            proj_k(qb, xn)
            proj_q(qb, xn, wq_t)
            proj_v(qb, xn, wv_t)
        produce_kb(0, kb_a)

    @pl.when(step < NAS)
    def _():
        h0 = step * HPS
        items = [(u, qb) for u in range(HPS) for qb in range(NQ)]
        kbs = [kb_a, kb_b]
        qms, qbv, blk, acc, lacc, vout = {}, {}, {}, {}, {}, {}
        chunks = [(it, c) for it in range(len(items)) for c in range(NC)]
        vpieces = [(it, c, lt, hf) for (it, c) in chunks if RV[c] for lt in range(NLT) for hf in range(2)]
        st = {"bad": None, "vi": 0, "cur": None, "tok": None, "sid": 0}
        links = {}

        def add_bad(b):
            st["bad"] = b if st["bad"] is None else jnp.maximum(st["bad"], b)

        def emit_vpiece():
            if st["vi"] >= len(vpieces):
                return
            it, c, lt, hf = vpieces[st["vi"]]
            st["vi"] += 1
            u, qb = items[it]
            if it not in qbv:
                q16 = qt_scr[qb, pl.ds(pl.multiple_of((h0 + u) * DH, DH), DH), :].astype(f32)
                qbv[it] = [jnp.broadcast_to(q16[d:d + 1, :], (8, BQ)) for d in range(DH)]
            if hf == 0:
                st["sid"] = (st["vi"] // 2) % NTH
                lk = links.get(st["sid"])
                a = None if lk is None else lk - lk
            else:
                a = st["cur"]
            for d in range(hf * 8, hf * 8 + 8):
                kbd = kbs[u % 2][d, pl.ds(VSTART[c], RV[c]), :]
                qbb = jnp.concatenate([qbv[it][d][:, lt * 128:(lt + 1) * 128]] * (RV[c] // 8), axis=0)
                term = kbd * qbb
                a = term if a is None else a + term
            st["cur"] = a
            if hf == 1:
                vout.setdefault((it, c), []).append(a)
                links[st["sid"]] = a

        def sum_add(it, p16, j):
            s2 = p16[0:8] + p16[8:16]
            key = (it, j % 2)
            lacc[key] = s2 if key not in lacc else lacc[key] + s2

        def emit_pv(ci):
            it, c = chunks[ci]
            u, qb = items[it]
            if c == 1 and qb == 0:
                produce_kb(jnp.minimum(h0 + u + 1, H - 1), kbs[(u + 1) % 2])
            while RV[c] and len(vout.get((it, c), [])) < NLT:
                emit_vpiece()
            target = len([cc for cc in chunks[:ci + 1 + VAHEAD] if RV[cc[1]]]) * NLT * 2
            todo = max(target - st["vi"], 0)
            ps = []
            if RV[c]:
                pvv = jnp.exp2(jnp.concatenate(vout.pop((it, c)), axis=1))
                sum_add(it, pvv, 0)
            for b in range(BPC[c]):
                p16 = jnp.exp2(blk.pop((it, MSTART[c] + b)))
                sum_add(it, p16, b + 1)
                ps.append(p16)
                for _ in range((todo * (b + 1)) // BPC[c] - (todo * b) // BPC[c]):
                    emit_vpiece()
            ps = ps[::-1]
            if RV[c]:
                ps.append(pvv)
            p = jnp.concatenate(ps, axis=0)
            if ci == len(chunks) - 1:
                p_def[...] = p
                acc_def[...] = acc.pop(it)
                l_def[...] = lacc.pop((it, 0)) + lacc.pop((it, 1))
                return
            pv = jnp.dot(vt_scr[h0 + u, :, pl.ds(c * C, C)], p, preferred_element_type=f32)
            z = pv[0:8, 0:128] - pv[0:8, 0:128]
            t = z if st["tok"] is None else st["tok"] + z
            st["tok"] = pltpu.roll(t, 1, 1) if TOKP[ci % len(TOKP)] == "r" else t
            acc[it] = pv if c == 0 else acc[it] + pv
            if c == NC - 1:
                o, bad = _normalise(acc.pop(it), lacc.pop((it, 0)) + lacc.pop((it, 1)))
                add_bad(bad)
                ot_scr[qb, pl.ds(pl.multiple_of((h0 + u) * DH, DH), DH), :] = o

        add_bad(deferred_pv(jnp.maximum(h0 - 1, 0)))
        pvi = 0
        for it, (u, qb) in enumerate(items):
            qms[it] = masked_qt(h0 + u, qb)
            bounds = sorted(set([0, NB] + [MSTART[c] + OFFB for c in range(NC) if MSTART[c] + OFFB < NB]))
            for a, b in zip(bounds[:-1], bounds[1:]):
                sm = jnp.dot(k_rows((h0 + u) // 8, a, b - a), qms[it], preferred_element_type=f32)
                for j in range(a, b):
                    blk[(it, j)] = sm[(j - a) * 16:(j - a + 1) * 16]
                pos = it * NB + b
                while pvi < len(chunks):
                    cit, cc = chunks[pvi]
                    nxt = cc + 2
                    need = cit * NB + MSTART[nxt] if nxt <= NC else (cit + 1) * NB + MSTART[nxt - NC]
                    if need + OFFB > pos:
                        break
                    emit_pv(pvi)
                    pvi += 1
        while pvi < len(chunks):
            emit_pv(pvi)
            pvi += 1
        tok_bad = jnp.where(st["tok"] == 0.0, 0.0, 1.0)
        add_bad(jnp.concatenate([tok_bad] * NLT, axis=1))
        bad_scr[...] = jnp.maximum(bad_scr[...], st["bad"])

    @pl.when(step == NAS)
    def _():
        for j in range(len(late)):
            late_copy(j).wait()
        bad = jnp.maximum(bad_scr[...], deferred_pv(H - 1))

        @pl.when(jnp.max(bad) > 0.0)
        def _():
            def body(i, carry):
                h = i // NQ
                qb = i % NQ
                qm = masked_qt(h, qb)
                sm = jnp.dot(k_rows(h // 8, 0, NB), qm, preferred_element_type=f32)
                sv = jnp.dot(kv_scr[h // 8].astype(bf16), qm, preferred_element_type=f32)
                m = jnp.maximum(jnp.max(sm, axis=0, keepdims=True), jnp.max(sv, axis=0, keepdims=True))
                pm = jnp.exp2(sm - m)
                pvv = jnp.exp2(sv - m)
                l = jnp.sum(pm, axis=0, keepdims=True) + jnp.sum(pvv, axis=0, keepdims=True)
                parts = []
                for c in range(NC):
                    for b in range(BPC[c]):
                        j = MSTART[c] + BPC[c] - 1 - b
                        parts.append(pm[j * 16:(j + 1) * 16])
                    if RV[c]:
                        parts.append(pvv[VSTART[c]:VSTART[c] + RV[c]])
                pn = jnp.concatenate(parts, axis=0)
                a = jnp.dot(vt_scr[h], pn, preferred_element_type=f32)
                ot_scr[qb, pl.ds(pl.multiple_of(h * DH, DH), DH), :] = (a * (1.0 / l)).astype(bf16)
                return carry
            lax.fori_loop(0, H * NQ, body, 0)

    @pl.when(step >= NAS)
    def _():
        fb = step - NAS
        rng = range(FSUB)
        r0 = [pl.multiple_of(fb * BQ + j * SUB, SUB) for j in rng]
        o = [ot_scr[fb, :, pl.ds(j * SUB, SUB)].astype(f32).T.astype(bf16) for j in rng]
        h1 = [x_v[pl.ds(r0[j], SUB), :].astype(f32) + jnp.dot(o[j], wo_v[...], preferred_element_type=f32)
              for j in rng]
        hn = [_ln(h1[j]).astype(bf16) for j in rng]
        act = []
        for j in rng:
            gate = lax.dot_general(hn[j], w1t_v[...], NT, preferred_element_type=f32)
            up = lax.dot_general(hn[j], w3t_v[...], NT, preferred_element_type=f32)
            act.append((gate * jax.nn.sigmoid(gate) * up).astype(bf16))
        for j in rng:
            out = h1[j] + jnp.dot(act[j], w2_v[...], preferred_element_type=f32)
            out_v[pl.ds(r0[j], SUB), :] = out.astype(bf16)
            out_copy(r0[j], fb * FSUB + j).start()

    @pl.when(step == NAS + NQ - 1)
    def _():
        for i in range(NQ * FSUB):
            out_copy(i * SUB, i).wait()


@jax.jit
def pallas_sequential_preLN__softmax_full_mha__glu_gated_swiglu__prompt_kernel(
    A_x: jax.Array,
    A_wqkv: jax.Array,
    A_wo: jax.Array,
    B_x: jax.Array,
    B_w1: jax.Array,
    B_w3: jax.Array,
    B_w2: jax.Array,
):
    hbm = pl.BlockSpec(memory_space=pl.ANY)
    out = pl.pallas_call(
        _kernel,
        grid=(NAS + NQ,),
        in_specs=[hbm] * 6,
        out_specs=hbm,
        out_shape=jax.ShapeDtypeStruct((S, D), bf16),
        scratch_shapes=[
            pltpu.VMEM((S, D), bf16),
            pltpu.VMEM((D, 3 * D), bf16),
            pltpu.VMEM((D, D), bf16),
            pltpu.VMEM((F, D), bf16),
            pltpu.VMEM((F, D), bf16),
            pltpu.VMEM((F, D), bf16),
            pltpu.VMEM((S, D), bf16),
            pltpu.VMEM((4, NBP * 8, 128), u32),
            pltpu.VMEM((4, NV, 128), f32),
            pltpu.VMEM((NQ, D, BQ), bf16),
            pltpu.VMEM((H, DH, S), f32),
            pltpu.VMEM((NQ, D, BQ), bf16),
            pltpu.VMEM((8, BQ), f32),
            pltpu.VMEM((DH, NV, 128), f32),
            pltpu.VMEM((DH, NV, 128), f32),
            pltpu.VMEM((C, BQ), f32),
            pltpu.VMEM((DH, BQ), f32),
            pltpu.VMEM((8, BQ), f32),
            pltpu.SemaphoreType.DMA((NQ + 3 + 4,)),
            pltpu.SemaphoreType.DMA((NQ * FSUB,)),
        ],
        compiler_params=pltpu.CompilerParams(dimension_semantics=("arbitrary",),
                                             vmem_limit_bytes=100 * 1024 * 1024),
    )(A_x.reshape(S, D), A_wqkv, A_wo, B_w1.T, B_w3.T, B_w2)
    return out.reshape(1, S, D)
```

```python
import jax
import jax.numpy as jnp
from jax import lax
from jax.experimental import pallas as pl
from jax.experimental.pallas import tpu as pltpu

S, D, H, DH, F = 2048, 512, 32, 16, 1376
LOG2E = 1.4426950408889634
EPS = 1e-5
f32, bf16, u32 = jnp.float32, jnp.bfloat16, jnp.uint32

BQ = 512
NQ = S // BQ
NLT = BQ // 128
C = 128
NC = S // C
HPS = 2
NAS = H // HPS
OFFB = 2
VAHEAD = 5
VPAT = (16,) * 15 + (0,)
NTH = 3
TOKP = "rr-"
FSUB = 4
SUB = BQ // FSUB
L_LO, L_HI, A_HI = 2.0 ** -40, 2.0 ** 60, 2.0 ** 100
NT = (((1,), (1,)), ((), ()))

RV = [VPAT[c % len(VPAT)] for c in range(NC)]
RM = [C - v for v in RV]
BPC = [r // 16 for r in RM]
MSTART = [sum(BPC[:c]) for c in range(NC + 1)]
VSTART = [sum(RV[:c]) for c in range(NC + 1)]
NB = MSTART[-1]
NBP = -(-NB // 4) * 4
NV = VSTART[-1]


def _ln(x):
    m = jnp.mean(x, axis=-1, keepdims=True)
    xc = x - m
    v = jnp.mean(xc * xc, axis=-1, keepdims=True)
    return xc * lax.rsqrt(v + EPS)


def _normalise(a, l8):
    l = jnp.sum(l8, axis=0, keepdims=True)
    ok_l = jnp.logical_and(l >= L_LO, l <= L_HI)
    bad_a = jnp.where(jnp.abs(a) <= A_HI, 0.0, 1.0)
    bad = jnp.maximum(jnp.maximum(bad_a[0:8], bad_a[8:16]), jnp.where(ok_l, 0.0, 1.0))
    return (a * (1.0 / l)).astype(bf16), bad


def _kernel(x_hbm, wqkv_hbm, wo_hbm, w1t_hbm, w3t_hbm, w2_hbm, o_hbm,
            x_v, wqkv_v, wo_v, w1t_v, w3t_v, w2_v, out_v,
            k_scr, kv_scr, qt_scr, vt_scr, ot_scr, bad_scr, kb_a, kb_b, p_def, acc_def, l_def, o_pre,
            sems, osems):
    step = pl.program_id(0)

    def x_copy(i):
        return pltpu.make_async_copy(x_hbm.at[pl.ds(i * BQ, BQ), :], x_v.at[pl.ds(i * BQ, BQ), :], sems.at[i])

    def w_copy(j):
        return pltpu.make_async_copy(wqkv_hbm.at[:, pl.ds(j * D, D)], wqkv_v.at[:, pl.ds(j * D, D)], sems.at[NQ + j])

    late = [(wo_hbm, wo_v), (w1t_hbm, w1t_v), (w3t_hbm, w3t_v), (w2_hbm, w2_v)]

    def late_copy(j):
        return pltpu.make_async_copy(late[j][0], late[j][1], sems.at[NQ + 3 + j])

    def out_copy(r0, i):
        return pltpu.make_async_copy(out_v.at[pl.ds(r0, SUB), :], o_hbm.at[pl.ds(r0, SUB), :], osems.at[i])

    def k_rows(g, blk0, nblk):
        return pltpu.bitcast(k_scr[g, pl.ds(blk0 * 8, nblk * 8), :], bf16)

    def masked_qt(h, qb):
        qt = qt_scr[qb, pl.ds(pl.multiple_of((h // 8) * 128, 128), 128), :]
        rows = lax.broadcasted_iota(jnp.int32, (128, BQ), 0) // DH
        return jnp.where(rows == h % 8, qt.astype(f32), 0.0).astype(bf16)

    def produce_kb(h, kb):
        x = pltpu.roll(kv_scr[h // 8], (128 - (h % 8) * DH) % 128, 1)
        for d in range(DH):
            kb[d] = jnp.broadcast_to(x[:, d:d + 1], (NV, 128))

    def o_rows(fb, j):
        return ot_scr[fb, :, pl.ds(j * SUB, SUB)].astype(f32).T.astype(bf16)

    def deferred_pv(h):
        a = acc_def[...] + jnp.dot(vt_scr[h, :, pl.ds((NC - 1) * C, C)], p_def[...], preferred_element_type=f32)
        o, bad = _normalise(a, l_def[...])
        ot_scr[NQ - 1, pl.ds(pl.multiple_of(h * DH, DH), DH), :] = o
        return bad

    @pl.when(step == 0)
    def _():
        x_copy(0).start()
        w_copy(1).start()
        w_copy(0).start()
        w_copy(2).start()
        for i in range(1, NQ):
            x_copy(i).start()
        bad_scr[...] = jnp.zeros_like(bad_scr)
        p_def[...] = jnp.zeros_like(p_def)
        acc_def[...] = jnp.zeros_like(acc_def)
        l_def[...] = jnp.ones_like(l_def)

        def proj_k(qb, xn):
            k = jnp.dot(xn, wqkv_v[:, D:2 * D], preferred_element_type=f32).astype(bf16)
            for cc in range(BQ // C):
                c = qb * (BQ // C) + cc
                for b in range(BPC[c]):
                    r0 = cc * C + (BPC[c] - 1 - b) * 16
                    for g in range(4):
                        k_scr[g, pl.ds((MSTART[c] + b) * 8, 8), :] = pltpu.bitcast(
                            k[r0:r0 + 16, g * 128:(g + 1) * 128], u32)
                if RV[c]:
                    r0 = cc * C + RM[c]
                    kf = k[r0:r0 + RV[c]].astype(f32)
                    for g in range(4):
                        kv_scr[g, pl.ds(VSTART[c], RV[c]), :] = kf[:, g * 128:(g + 1) * 128]

        def proj_q(qb, xn, wq_t):
            qt = lax.dot_general(wq_t, xn, NT, preferred_element_type=f32)
            qt_scr[qb] = (qt * (DH ** -0.5 * LOG2E)).astype(bf16)

        def proj_v(qb, xn, wv_t):
            vt = lax.dot_general(wv_t, xn, NT, preferred_element_type=f32)
            vt_scr[:, :, pl.ds(qb * BQ, BQ)] = vt.astype(bf16).astype(f32).reshape(H, DH, BQ)

        def ln_chunk(qb):
            return _ln(x_v[pl.ds(qb * BQ, BQ), :].astype(f32)).astype(bf16)

        x_copy(0).wait()
        xn0 = ln_chunk(0)
        w_copy(1).wait()
        proj_k(0, xn0)
        w_copy(0).wait()
        wq_t = wqkv_v[:, 0:D].astype(f32).T.astype(bf16)
        proj_q(0, xn0, wq_t)
        for j in range(len(late)):
            late_copy(j).start()
        w_copy(2).wait()
        x_copy(1).wait()
        wv_t = wqkv_v[:, 2 * D:3 * D].astype(f32).T.astype(bf16)
        xn1 = ln_chunk(1)
        proj_v(0, xn0, wv_t)
        for i in range(2, NQ):
            x_copy(i).wait()
        for qb in range(1, NQ):
            xn = xn1 if qb == 1 else ln_chunk(qb)
            proj_k(qb, xn)
            proj_q(qb, xn, wq_t)
            proj_v(qb, xn, wv_t)
        produce_kb(0, kb_a)

    @pl.when(step < NAS)
    def _():
        h0 = step * HPS
        items = [(u, qb) for u in range(HPS) for qb in range(NQ)]
        kbs = [kb_a, kb_b]
        qms, qbv, blk, acc, lacc, vout = {}, {}, {}, {}, {}, {}
        chunks = [(it, c) for it in range(len(items)) for c in range(NC)]
        vpieces = [(it, c, lt, hf) for (it, c) in chunks if RV[c] for lt in range(NLT) for hf in range(2)]
        st = {"bad": None, "vi": 0, "cur": None, "tok": None, "sid": 0}
        links = {}

        def add_bad(b):
            st["bad"] = b if st["bad"] is None else jnp.maximum(st["bad"], b)

        def emit_vpiece():
            if st["vi"] >= len(vpieces):
                return
            it, c, lt, hf = vpieces[st["vi"]]
            st["vi"] += 1
            u, qb = items[it]
            if it not in qbv:
                q16 = qt_scr[qb, pl.ds(pl.multiple_of((h0 + u) * DH, DH), DH), :].astype(f32)
                qbv[it] = [jnp.broadcast_to(q16[d:d + 1, :], (8, BQ)) for d in range(DH)]
            if hf == 0:
                st["sid"] = (st["vi"] // 2) % NTH
                lk = links.get(st["sid"])
                a = None if lk is None else lk - lk
            else:
                a = st["cur"]
            for d in range(hf * 8, hf * 8 + 8):
                kbd = kbs[u % 2][d, pl.ds(VSTART[c], RV[c]), :]
                qbb = jnp.concatenate([qbv[it][d][:, lt * 128:(lt + 1) * 128]] * (RV[c] // 8), axis=0)
                term = kbd * qbb
                a = term if a is None else a + term
            st["cur"] = a
            if hf == 1:
                vout.setdefault((it, c), []).append(a)
                links[st["sid"]] = a

        def sum_add(it, p16, j):
            s2 = p16[0:8] + p16[8:16]
            key = (it, j % 2)
            lacc[key] = s2 if key not in lacc else lacc[key] + s2

        def emit_pv(ci):
            it, c = chunks[ci]
            u, qb = items[it]
            if c == 3 and qb == 1:
                produce_kb(jnp.minimum(h0 + u + 1, H - 1), kbs[(u + 1) % 2])
            while RV[c] and len(vout.get((it, c), [])) < NLT:
                emit_vpiece()
            target = len([cc for cc in chunks[:ci + 1 + VAHEAD] if RV[cc[1]]]) * NLT * 2
            todo = max(target - st["vi"], 0)
            ps = []
            if RV[c]:
                pvv = jnp.exp2(jnp.concatenate(vout.pop((it, c)), axis=1))
                sum_add(it, pvv, 0)
            for b in range(BPC[c]):
                p16 = jnp.exp2(blk.pop((it, MSTART[c] + b)))
                sum_add(it, p16, b + 1)
                ps.append(p16)
                for _ in range((todo * (b + 1)) // BPC[c] - (todo * b) // BPC[c]):
                    emit_vpiece()
            ps = ps[::-1]
            if RV[c]:
                ps.append(pvv)
            p = jnp.concatenate(ps, axis=0)
            if ci == len(chunks) - 1:
                p_def[...] = p
                acc_def[...] = acc.pop(it)
                l_def[...] = lacc.pop((it, 0)) + lacc.pop((it, 1))
                return
            pv = jnp.dot(vt_scr[h0 + u, :, pl.ds(c * C, C)], p, preferred_element_type=f32)
            z = pv[0:8, 0:128] - pv[0:8, 0:128]
            t = z if st["tok"] is None else st["tok"] + z
            st["tok"] = pltpu.roll(t, 1, 1) if TOKP[ci % len(TOKP)] == "r" else t
            acc[it] = pv if c == 0 else acc[it] + pv
            if c == NC - 1:
                o, bad = _normalise(acc.pop(it), lacc.pop((it, 0)) + lacc.pop((it, 1)))
                add_bad(bad)
                ot_scr[qb, pl.ds(pl.multiple_of((h0 + u) * DH, DH), DH), :] = o

        add_bad(deferred_pv(jnp.maximum(h0 - 1, 0)))
        pvi = 0
        for it, (u, qb) in enumerate(items):
            qms[it] = masked_qt(h0 + u, qb)
            bounds = sorted(set([0, NB] + [MSTART[c] + OFFB for c in range(NC) if MSTART[c] + OFFB < NB]))
            for a, b in zip(bounds[:-1], bounds[1:]):
                sm = jnp.dot(k_rows((h0 + u) // 8, a, b - a), qms[it], preferred_element_type=f32)
                for j in range(a, b):
                    blk[(it, j)] = sm[(j - a) * 16:(j - a + 1) * 16]
                pos = it * NB + b
                while pvi < len(chunks):
                    cit, cc = chunks[pvi]
                    nxt = cc + 2
                    need = cit * NB + MSTART[nxt] if nxt <= NC else (cit + 1) * NB + MSTART[nxt - NC]
                    if need + OFFB > pos:
                        break
                    emit_pv(pvi)
                    pvi += 1
        while pvi < len(chunks):
            emit_pv(pvi)
            pvi += 1
        tok_bad = jnp.where(st["tok"] == 0.0, 0.0, 1.0)
        add_bad(jnp.concatenate([tok_bad] * NLT, axis=1))
        bad_scr[...] = jnp.maximum(bad_scr[...], st["bad"])

    @pl.when(step == NAS)
    def _():
        for j in range(len(late)):
            late_copy(j).wait()
        bad = jnp.maximum(bad_scr[...], deferred_pv(H - 1))

        @pl.when(jnp.max(bad) > 0.0)
        def _():
            def body(i, carry):
                h = i // NQ
                qb = i % NQ
                qm = masked_qt(h, qb)
                sm = jnp.dot(k_rows(h // 8, 0, NB), qm, preferred_element_type=f32)
                sv = jnp.dot(kv_scr[h // 8].astype(bf16), qm, preferred_element_type=f32)
                m = jnp.maximum(jnp.max(sm, axis=0, keepdims=True), jnp.max(sv, axis=0, keepdims=True))
                pm = jnp.exp2(sm - m)
                pvv = jnp.exp2(sv - m)
                l = jnp.sum(pm, axis=0, keepdims=True) + jnp.sum(pvv, axis=0, keepdims=True)
                parts = []
                for c in range(NC):
                    for b in range(BPC[c]):
                        j = MSTART[c] + BPC[c] - 1 - b
                        parts.append(pm[j * 16:(j + 1) * 16])
                    if RV[c]:
                        parts.append(pvv[VSTART[c]:VSTART[c] + RV[c]])
                pn = jnp.concatenate(parts, axis=0)
                a = jnp.dot(vt_scr[h], pn, preferred_element_type=f32)
                ot_scr[qb, pl.ds(pl.multiple_of(h * DH, DH), DH), :] = (a * (1.0 / l)).astype(bf16)
                return carry
            lax.fori_loop(0, H * NQ, body, 0)

        o_pre[...] = o_rows(0, 0)

    @pl.when(step >= NAS)
    def _():
        fb = step - NAS
        rng = range(FSUB)
        r0 = [pl.multiple_of(fb * BQ + j * SUB, SUB) for j in rng]
        o = [o_pre[...] if j == 0 else o_rows(fb, j) for j in rng]
        h1 = [x_v[pl.ds(r0[j], SUB), :].astype(f32) + jnp.dot(o[j], wo_v[...], preferred_element_type=f32)
              for j in rng]
        hn = [_ln(h1[j]).astype(bf16) for j in rng]
        act = []
        for j in rng:
            gate = lax.dot_general(w1t_v[...], hn[j], NT, preferred_element_type=f32)
            up = lax.dot_general(w3t_v[...], hn[j], NT, preferred_element_type=f32)
            act.append((gate * jax.nn.sigmoid(gate) * up).T.astype(bf16))
        for j in rng:
            out = h1[j] + jnp.dot(act[j], w2_v[...], preferred_element_type=f32)
            out_v[pl.ds(r0[j], SUB), :] = out.astype(bf16)
            out_copy(r0[j], fb * FSUB + j).start()
        o_pre[...] = o_rows(jnp.minimum(fb + 1, NQ - 1), 0)

    @pl.when(step == NAS + NQ - 1)
    def _():
        for i in range(NQ * FSUB):
            out_copy(i * SUB, i).wait()


@jax.jit
def pallas_sequential_preLN__softmax_full_mha__glu_gated_swiglu__prompt_kernel(
    A_x: jax.Array,
    A_wqkv: jax.Array,
    A_wo: jax.Array,
    B_x: jax.Array,
    B_w1: jax.Array,
    B_w3: jax.Array,
    B_w2: jax.Array,
):
    hbm = pl.BlockSpec(memory_space=pl.ANY)
    out = pl.pallas_call(
        _kernel,
        grid=(NAS + NQ,),
        in_specs=[hbm] * 6,
        out_specs=hbm,
        out_shape=jax.ShapeDtypeStruct((S, D), bf16),
        scratch_shapes=[
            pltpu.VMEM((S, D), bf16),
            pltpu.VMEM((D, 3 * D), bf16),
            pltpu.VMEM((D, D), bf16),
            pltpu.VMEM((F, D), bf16),
            pltpu.VMEM((F, D), bf16),
            pltpu.VMEM((F, D), bf16),
            pltpu.VMEM((S, D), bf16),
            pltpu.VMEM((4, NBP * 8, 128), u32),
            pltpu.VMEM((4, NV, 128), f32),
            pltpu.VMEM((NQ, D, BQ), bf16),
            pltpu.VMEM((H, DH, S), f32),
            pltpu.VMEM((NQ, D, BQ), bf16),
            pltpu.VMEM((8, BQ), f32),
            pltpu.VMEM((DH, NV, 128), f32),
            pltpu.VMEM((DH, NV, 128), f32),
            pltpu.VMEM((C, BQ), f32),
            pltpu.VMEM((DH, BQ), f32),
            pltpu.VMEM((8, BQ), f32),
            pltpu.VMEM((SUB, D), bf16),
            pltpu.SemaphoreType.DMA((NQ + 3 + 4,)),
            pltpu.SemaphoreType.DMA((NQ * FSUB,)),
        ],
        compiler_params=pltpu.CompilerParams(dimension_semantics=("arbitrary",),
                                             vmem_limit_bytes=100 * 1024 * 1024),
    )(A_x.reshape(S, D), A_wqkv, A_wo, B_w1.T, B_w3.T, B_w2)
    return out.reshape(1, S, D)
```

```python
import jax
import jax.numpy as jnp
from jax import lax
from jax.experimental import pallas as pl
from jax.experimental.pallas import tpu as pltpu

S, D, H, DH, F = 2048, 512, 32, 16, 1376
LOG2E = 1.4426950408889634
EPS = 1e-5
f32, bf16, u32 = jnp.float32, jnp.bfloat16, jnp.uint32

BQ = 512
NQ = S // BQ
NLT = BQ // 128
C = 128
NC = S // C
HPS = 2
NAS = H // HPS
OFFB = 2
VAHEAD = 5
VPAT = (16,) * 15 + (0,)
NTH = 3
TOKP = "rr-"
FSUB = 4
SUB = BQ // FSUB
L_LO, L_HI, A_HI = 2.0 ** -40, 2.0 ** 60, 2.0 ** 100
NT = (((1,), (1,)), ((), ()))

RV = [VPAT[c % len(VPAT)] for c in range(NC)]
RM = [C - v for v in RV]
BPC = [r // 16 for r in RM]
MSTART = [sum(BPC[:c]) for c in range(NC + 1)]
VSTART = [sum(RV[:c]) for c in range(NC + 1)]
NB = MSTART[-1]
NBP = -(-NB // 4) * 4
NV = VSTART[-1]


def _ln(x):
    m = jnp.mean(x, axis=-1, keepdims=True)
    xc = x - m
    v = jnp.mean(xc * xc, axis=-1, keepdims=True)
    return xc * lax.rsqrt(v + EPS)


def _normalise(a, l8):
    l = jnp.sum(l8, axis=0, keepdims=True)
    ok_l = jnp.logical_and(l >= L_LO, l <= L_HI)
    bad_a = jnp.where(jnp.abs(a) <= A_HI, 0.0, 1.0)
    bad = jnp.maximum(jnp.maximum(bad_a[0:8], bad_a[8:16]), jnp.where(ok_l, 0.0, 1.0))
    return (a * (1.0 / l)).astype(bf16), bad


def _kernel(x_hbm, wqkv_hbm, wo_hbm, w1t_hbm, w3t_hbm, w2_hbm, o_hbm,
            x_v, wqkv_v, wo_v, w1t_v, w3t_v, w2_v, out_v,
            k_scr, kv_scr, qt_scr, vt_scr, ot_scr, bad_scr, kb_a, kb_b, qb_first, p_def, acc_def, l_def, o_pre,
            sems, osems):
    step = pl.program_id(0)

    def x_copy(i):
        return pltpu.make_async_copy(x_hbm.at[pl.ds(i * BQ, BQ), :], x_v.at[pl.ds(i * BQ, BQ), :], sems.at[i])

    def w_copy(j):
        return pltpu.make_async_copy(wqkv_hbm.at[:, pl.ds(j * D, D)], wqkv_v.at[:, pl.ds(j * D, D)], sems.at[NQ + j])

    late = [(wo_hbm, wo_v), (w1t_hbm, w1t_v), (w3t_hbm, w3t_v), (w2_hbm, w2_v)]

    def late_copy(j):
        return pltpu.make_async_copy(late[j][0], late[j][1], sems.at[NQ + 3 + j])

    def out_copy(r0, i):
        return pltpu.make_async_copy(out_v.at[pl.ds(r0, SUB), :], o_hbm.at[pl.ds(r0, SUB), :], osems.at[i])

    def k_rows(g, blk0, nblk):
        return pltpu.bitcast(k_scr[g, pl.ds(blk0 * 8, nblk * 8), :], bf16)

    def masked_qt(h, qb):
        qt = qt_scr[qb, pl.ds(pl.multiple_of((h // 8) * 128, 128), 128), :]
        rows = lax.broadcasted_iota(jnp.int32, (128, BQ), 0) // DH
        return jnp.where(rows == h % 8, qt.astype(f32), 0.0).astype(bf16)

    def produce_kb(h, kb):
        x = pltpu.roll(kv_scr[h // 8], (128 - (h % 8) * DH) % 128, 1)
        for d in range(DH):
            kb[d] = jnp.broadcast_to(x[:, d:d + 1], (NV, 128))

    def q_bcast(h, qb):
        q16 = qt_scr[qb, pl.ds(pl.multiple_of(h * DH, DH), DH), :].astype(f32)
        return [jnp.broadcast_to(q16[d:d + 1, :], (8, BQ)) for d in range(DH)]

    def prep_q_first(h):
        for d, v in enumerate(q_bcast(h, 0)):
            qb_first[d] = v

    def o_rows(fb, j):
        return ot_scr[fb, :, pl.ds(j * SUB, SUB)].astype(f32).T.astype(bf16)

    def deferred_pv(h):
        a = acc_def[...] + jnp.dot(vt_scr[h, :, pl.ds((NC - 1) * C, C)], p_def[...], preferred_element_type=f32)
        o, bad = _normalise(a, l_def[...])
        ot_scr[NQ - 1, pl.ds(pl.multiple_of(h * DH, DH), DH), :] = o
        return bad

    @pl.when(step == 0)
    def _():
        x_copy(0).start()
        w_copy(1).start()
        w_copy(0).start()
        w_copy(2).start()
        for i in range(1, NQ):
            x_copy(i).start()
        bad_scr[...] = jnp.zeros_like(bad_scr)
        p_def[...] = jnp.zeros_like(p_def)
        acc_def[...] = jnp.zeros_like(acc_def)
        l_def[...] = jnp.ones_like(l_def)

        def proj_k(qb, xn):
            k = jnp.dot(xn, wqkv_v[:, D:2 * D], preferred_element_type=f32).astype(bf16)
            for cc in range(BQ // C):
                c = qb * (BQ // C) + cc
                for b in range(BPC[c]):
                    r0 = cc * C + (BPC[c] - 1 - b) * 16
                    for g in range(4):
                        k_scr[g, pl.ds((MSTART[c] + b) * 8, 8), :] = pltpu.bitcast(
                            k[r0:r0 + 16, g * 128:(g + 1) * 128], u32)
                if RV[c]:
                    r0 = cc * C + RM[c]
                    kf = k[r0:r0 + RV[c]].astype(f32)
                    for g in range(4):
                        kv_scr[g, pl.ds(VSTART[c], RV[c]), :] = kf[:, g * 128:(g + 1) * 128]

        def proj_q(qb, xn, wq_t):
            qt = lax.dot_general(wq_t, xn, NT, preferred_element_type=f32)
            qt_scr[qb] = (qt * (DH ** -0.5 * LOG2E)).astype(bf16)

        def proj_v(qb, xn, wv_t):
            vt = lax.dot_general(wv_t, xn, NT, preferred_element_type=f32)
            vt_scr[:, :, pl.ds(qb * BQ, BQ)] = vt.astype(bf16).astype(f32).reshape(H, DH, BQ)

        def ln_chunk(qb):
            return _ln(x_v[pl.ds(qb * BQ, BQ), :].astype(f32)).astype(bf16)

        x_copy(0).wait()
        xn0 = ln_chunk(0)
        w_copy(1).wait()
        proj_k(0, xn0)
        w_copy(0).wait()
        w_copy(2).wait()
        wq_t = wqkv_v[:, 0:D].astype(f32).T.astype(bf16)
        wv_t = wqkv_v[:, 2 * D:3 * D].astype(f32).T.astype(bf16)
        proj_q(0, xn0, wq_t)
        for j in range(len(late)):
            late_copy(j).start()
        x_copy(1).wait()
        xn1 = ln_chunk(1)
        proj_v(0, xn0, wv_t)
        for i in range(2, NQ):
            x_copy(i).wait()
        for qb in range(1, NQ):
            xn = xn1 if qb == 1 else ln_chunk(qb)
            proj_k(qb, xn)
            proj_q(qb, xn, wq_t)
            proj_v(qb, xn, wv_t)
        produce_kb(0, kb_a)
        prep_q_first(0)

    @pl.when(step < NAS)
    def _():
        h0 = step * HPS
        items = [(u, qb) for u in range(HPS) for qb in range(NQ)]
        kbs = [kb_a, kb_b]
        qms, qbv, blk, acc, lacc, vout = {}, {}, {}, {}, {}, {}
        chunks = [(it, c) for it in range(len(items)) for c in range(NC)]
        vpieces = [(it, c, lt, hf) for (it, c) in chunks if RV[c] for lt in range(NLT) for hf in range(2)]
        st = {"bad": None, "vi": 0, "cur": None, "tok": None, "sid": 0}
        links = {}

        def add_bad(b):
            st["bad"] = b if st["bad"] is None else jnp.maximum(st["bad"], b)

        def emit_vpiece():
            if st["vi"] >= len(vpieces):
                return
            it, c, lt, hf = vpieces[st["vi"]]
            st["vi"] += 1
            u, qb = items[it]
            if it not in qbv:
                qbv[it] = [qb_first[d] for d in range(DH)] if it == 0 else q_bcast(h0 + u, qb)
            if hf == 0:
                st["sid"] = (st["vi"] // 2) % NTH
                lk = links.get(st["sid"])
                a = None if lk is None else lk - lk
            else:
                a = st["cur"]
            for d in range(hf * 8, hf * 8 + 8):
                kbd = kbs[u % 2][d, pl.ds(VSTART[c], RV[c]), :]
                qbb = jnp.concatenate([qbv[it][d][:, lt * 128:(lt + 1) * 128]] * (RV[c] // 8), axis=0)
                term = kbd * qbb
                a = term if a is None else a + term
            st["cur"] = a
            if hf == 1:
                vout.setdefault((it, c), []).append(a)
                links[st["sid"]] = a

        def sum_add(it, p16, j):
            s2 = p16[0:8] + p16[8:16]
            key = (it, j % 2)
            lacc[key] = s2 if key not in lacc else lacc[key] + s2

        def emit_pv(ci):
            it, c = chunks[ci]
            u, qb = items[it]
            if c == 3 and qb == 1:
                produce_kb(jnp.minimum(h0 + u + 1, H - 1), kbs[(u + 1) % 2])
            while RV[c] and len(vout.get((it, c), [])) < NLT:
                emit_vpiece()
            target = len([cc for cc in chunks[:ci + 1 + VAHEAD] if RV[cc[1]]]) * NLT * 2
            todo = max(target - st["vi"], 0)
            ps = []
            if RV[c]:
                pvv = jnp.exp2(jnp.concatenate(vout.pop((it, c)), axis=1))
                sum_add(it, pvv, 0)
            for b in range(BPC[c]):
                p16 = jnp.exp2(blk.pop((it, MSTART[c] + b)))
                sum_add(it, p16, b + 1)
                ps.append(p16)
                for _ in range((todo * (b + 1)) // BPC[c] - (todo * b) // BPC[c]):
                    emit_vpiece()
            ps = ps[::-1]
            if RV[c]:
                ps.append(pvv)
            p = jnp.concatenate(ps, axis=0)
            if ci == len(chunks) - 1:
                p_def[...] = p
                acc_def[...] = acc.pop(it)
                l_def[...] = lacc.pop((it, 0)) + lacc.pop((it, 1))
                return
            pv = jnp.dot(vt_scr[h0 + u, :, pl.ds(c * C, C)], p, preferred_element_type=f32)
            z = pv[0:8, 0:128] - pv[0:8, 0:128]
            t = z if st["tok"] is None else st["tok"] + z
            st["tok"] = pltpu.roll(t, 1, 1) if TOKP[ci % len(TOKP)] == "r" else t
            acc[it] = pv if c == 0 else acc[it] + pv
            if c == NC - 1:
                o, bad = _normalise(acc.pop(it), lacc.pop((it, 0)) + lacc.pop((it, 1)))
                add_bad(bad)
                ot_scr[qb, pl.ds(pl.multiple_of((h0 + u) * DH, DH), DH), :] = o

        add_bad(deferred_pv(jnp.maximum(h0 - 1, 0)))
        pvi = 0
        for it, (u, qb) in enumerate(items):
            qms[it] = masked_qt(h0 + u, qb)
            bounds = sorted(set([0, NB] + [MSTART[c] + OFFB for c in range(NC) if MSTART[c] + OFFB < NB]))
            for a, b in zip(bounds[:-1], bounds[1:]):
                sm = jnp.dot(k_rows((h0 + u) // 8, a, b - a), qms[it], preferred_element_type=f32)
                for j in range(a, b):
                    blk[(it, j)] = sm[(j - a) * 16:(j - a + 1) * 16]
                pos = it * NB + b
                while pvi < len(chunks):
                    cit, cc = chunks[pvi]
                    nxt = cc + 2
                    need = cit * NB + MSTART[nxt] if nxt <= NC else (cit + 1) * NB + MSTART[nxt - NC]
                    if need + OFFB > pos:
                        break
                    emit_pv(pvi)
                    pvi += 1
        while pvi < len(chunks):
            emit_pv(pvi)
            pvi += 1
        prep_q_first(jnp.minimum(h0 + HPS, H - 1))
        tok_bad = jnp.where(st["tok"] == 0.0, 0.0, 1.0)
        add_bad(jnp.concatenate([tok_bad] * NLT, axis=1))
        bad_scr[...] = jnp.maximum(bad_scr[...], st["bad"])

    @pl.when(step == NAS)
    def _():
        for j in range(len(late)):
            late_copy(j).wait()
        bad = jnp.maximum(bad_scr[...], deferred_pv(H - 1))
        o_pre[...] = o_rows(0, 0)

        @pl.when(jnp.max(bad) > 0.0)
        def _():
            def body(i, carry):
                h = i // NQ
                qb = i % NQ
                qm = masked_qt(h, qb)
                sm = jnp.dot(k_rows(h // 8, 0, NB), qm, preferred_element_type=f32)
                sv = jnp.dot(kv_scr[h // 8].astype(bf16), qm, preferred_element_type=f32)
                m = jnp.maximum(jnp.max(sm, axis=0, keepdims=True), jnp.max(sv, axis=0, keepdims=True))
                pm = jnp.exp2(sm - m)
                pvv = jnp.exp2(sv - m)
                l = jnp.sum(pm, axis=0, keepdims=True) + jnp.sum(pvv, axis=0, keepdims=True)
                parts = []
                for c in range(NC):
                    for b in range(BPC[c]):
                        j = MSTART[c] + BPC[c] - 1 - b
                        parts.append(pm[j * 16:(j + 1) * 16])
                    if RV[c]:
                        parts.append(pvv[VSTART[c]:VSTART[c] + RV[c]])
                pn = jnp.concatenate(parts, axis=0)
                a = jnp.dot(vt_scr[h], pn, preferred_element_type=f32)
                ot_scr[qb, pl.ds(pl.multiple_of(h * DH, DH), DH), :] = (a * (1.0 / l)).astype(bf16)
                return carry
            lax.fori_loop(0, H * NQ, body, 0)
            o_pre[...] = o_rows(0, 0)

    @pl.when(step >= NAS)
    def _():
        fb = step - NAS
        rng = range(FSUB)
        r0 = [pl.multiple_of(fb * BQ + j * SUB, SUB) for j in rng]
        o = [o_pre[...] if j == 0 else o_rows(fb, j) for j in rng]
        h1 = [x_v[pl.ds(r0[j], SUB), :].astype(f32) + jnp.dot(o[j], wo_v[...], preferred_element_type=f32)
              for j in rng]
        hn = [_ln(h1[j]).astype(bf16) for j in rng]
        act = []
        for j in rng:
            gate = lax.dot_general(w1t_v[...], hn[j], NT, preferred_element_type=f32)
            up = lax.dot_general(w3t_v[...], hn[j], NT, preferred_element_type=f32)
            act.append((gate * jax.nn.sigmoid(gate) * up).T.astype(bf16))
        for j in rng:
            out = h1[j] + jnp.dot(act[j], w2_v[...], preferred_element_type=f32)
            out_v[pl.ds(r0[j], SUB), :] = out.astype(bf16)
            out_copy(r0[j], fb * FSUB + j).start()
        o_pre[...] = o_rows(jnp.minimum(fb + 1, NQ - 1), 0)

    @pl.when(step == NAS + NQ - 1)
    def _():
        for i in range(NQ * FSUB):
            out_copy(i * SUB, i).wait()


@jax.jit
def pallas_sequential_preLN__softmax_full_mha__glu_gated_swiglu__prompt_kernel(
    A_x: jax.Array,
    A_wqkv: jax.Array,
    A_wo: jax.Array,
    B_x: jax.Array,
    B_w1: jax.Array,
    B_w3: jax.Array,
    B_w2: jax.Array,
):
    hbm = pl.BlockSpec(memory_space=pl.ANY)
    out = pl.pallas_call(
        _kernel,
        grid=(NAS + NQ,),
        in_specs=[hbm] * 6,
        out_specs=hbm,
        out_shape=jax.ShapeDtypeStruct((S, D), bf16),
        scratch_shapes=[
            pltpu.VMEM((S, D), bf16),
            pltpu.VMEM((D, 3 * D), bf16),
            pltpu.VMEM((D, D), bf16),
            pltpu.VMEM((F, D), bf16),
            pltpu.VMEM((F, D), bf16),
            pltpu.VMEM((F, D), bf16),
            pltpu.VMEM((S, D), bf16),
            pltpu.VMEM((4, NBP * 8, 128), u32),
            pltpu.VMEM((4, NV, 128), f32),
            pltpu.VMEM((NQ, D, BQ), bf16),
            pltpu.VMEM((H, DH, S), f32),
            pltpu.VMEM((NQ, D, BQ), bf16),
            pltpu.VMEM((8, BQ), f32),
            pltpu.VMEM((DH, NV, 128), f32),
            pltpu.VMEM((DH, NV, 128), f32),
            pltpu.VMEM((DH, 8, BQ), f32),
            pltpu.VMEM((C, BQ), f32),
            pltpu.VMEM((DH, BQ), f32),
            pltpu.VMEM((8, BQ), f32),
            pltpu.VMEM((SUB, D), bf16),
            pltpu.SemaphoreType.DMA((NQ + 3 + 4,)),
            pltpu.SemaphoreType.DMA((NQ * FSUB,)),
        ],
        compiler_params=pltpu.CompilerParams(dimension_semantics=("arbitrary",),
                                             vmem_limit_bytes=100 * 1024 * 1024),
    )(A_x.reshape(S, D), A_wqkv, A_wo, B_w1.T, B_w3.T, B_w2)
    return out.reshape(1, S, D)
```

```python
import jax
import jax.numpy as jnp
from jax import lax
from jax.experimental import pallas as pl
from jax.experimental.pallas import tpu as pltpu

S, D, H, DH, F = 2048, 512, 32, 16, 1376
LOG2E = 1.4426950408889634
EPS = 1e-5
f32, bf16, u32 = jnp.float32, jnp.bfloat16, jnp.uint32

BQ = 512
NQ = S // BQ
NLT = BQ // 128
C = 128
NC = S // C
HPS = 2
NAS = H // HPS
OFFB = 2
VAHEAD = 5
VPAT = (16,) * 15 + (0,)
NTH = 3
TOKP = "r-r"
FSUB = 4
SUB = BQ // FSUB
L_LO, L_HI, A_HI = 2.0 ** -40, 2.0 ** 100, 2.0 ** 120
NT = (((1,), (1,)), ((), ()))

RV = [VPAT[c % len(VPAT)] for c in range(NC)]
RM = [C - v for v in RV]
BPC = [r // 16 for r in RM]
MSTART = [sum(BPC[:c]) for c in range(NC + 1)]
VSTART = [sum(RV[:c]) for c in range(NC + 1)]
NB = MSTART[-1]
NBP = -(-NB // 4) * 4
NV = VSTART[-1]


def _ln(x):
    m = jnp.mean(x, axis=-1, keepdims=True)
    xc = x - m
    v = jnp.mean(xc * xc, axis=-1, keepdims=True)
    return xc * lax.rsqrt(v + EPS)


def _pv_dot(vt, p):
    return jnp.dot(vt, p, precision=lax.Precision.DEFAULT, preferred_element_type=f32)


def _normalise(a, l8):
    l = jnp.sum(l8, axis=0, keepdims=True)
    ok_l = jnp.logical_and(l >= L_LO, l <= L_HI)
    bad_a = jnp.where(jnp.abs(a) <= A_HI, 0.0, 1.0)
    bad = jnp.maximum(jnp.maximum(bad_a[0:8], bad_a[8:16]), jnp.where(ok_l, 0.0, 1.0))
    return (a * (1.0 / l)).astype(bf16), bad


def _kernel(x_hbm, wqkv_hbm, wo_hbm, w1t_hbm, w3t_hbm, w2_hbm, o_hbm,
            x_v, wqkv_v, wo_v, w1t_v, w3t_v, w2_v, out_v,
            k_scr, kv_scr, qt_scr, vt_scr, ot_scr, bad_scr, kb_a, kb_b, qb_first, p_def, acc_def, l_def, o_pre,
            sems, osems):
    step = pl.program_id(0)

    def x_copy(i):
        return pltpu.make_async_copy(x_hbm.at[pl.ds(i * BQ, BQ), :], x_v.at[pl.ds(i * BQ, BQ), :], sems.at[i])

    def w_copy(j):
        return pltpu.make_async_copy(wqkv_hbm.at[:, pl.ds(j * D, D)], wqkv_v.at[:, pl.ds(j * D, D)], sems.at[NQ + j])

    late = [(wo_hbm, wo_v), (w1t_hbm, w1t_v), (w3t_hbm, w3t_v), (w2_hbm, w2_v)]

    def late_copy(j):
        return pltpu.make_async_copy(late[j][0], late[j][1], sems.at[NQ + 3 + j])

    def out_copy(r0, i):
        return pltpu.make_async_copy(out_v.at[pl.ds(r0, SUB), :], o_hbm.at[pl.ds(r0, SUB), :], osems.at[i])

    def k_rows(g, blk0, nblk):
        return pltpu.bitcast(k_scr[g, pl.ds(blk0 * 8, nblk * 8), :], bf16)

    def masked_qt(h, qb):
        qt = qt_scr[qb, pl.ds(pl.multiple_of((h // 8) * 128, 128), 128), :]
        rows = lax.broadcasted_iota(jnp.int32, (128, BQ), 0) // DH
        return jnp.where(rows == h % 8, qt.astype(f32), 0.0).astype(bf16)

    def produce_kb(h, kb):
        x = pltpu.roll(kv_scr[h // 8], (128 - (h % 8) * DH) % 128, 1)
        for d in range(DH):
            kb[d] = jnp.broadcast_to(x[:, d:d + 1], (NV, 128))

    def q_bcast(h, qb):
        q16 = qt_scr[qb, pl.ds(pl.multiple_of(h * DH, DH), DH), :].astype(f32)
        return [jnp.broadcast_to(q16[d:d + 1, :], (8, BQ)) for d in range(DH)]

    def prep_q_first(h):
        for d, v in enumerate(q_bcast(h, 0)):
            qb_first[d] = v

    def o_rows(fb, j):
        return ot_scr[fb, :, pl.ds(j * SUB, SUB)].astype(f32).T.astype(bf16)

    def deferred_pv(h):
        a = acc_def[...] + _pv_dot(vt_scr[h, :, pl.ds((NC - 1) * C, C)], p_def[...])
        o, bad = _normalise(a, l_def[...])
        ot_scr[NQ - 1, pl.ds(pl.multiple_of(h * DH, DH), DH), :] = o
        return bad

    @pl.when(step == 0)
    def _():
        x_copy(0).start()
        w_copy(1).start()
        w_copy(0).start()
        w_copy(2).start()
        for i in range(1, NQ):
            x_copy(i).start()
        bad_scr[...] = jnp.zeros_like(bad_scr)
        p_def[...] = jnp.zeros_like(p_def)
        acc_def[...] = jnp.zeros_like(acc_def)
        l_def[...] = jnp.ones_like(l_def)

        def proj_k(qb, xn):
            k = jnp.dot(xn, wqkv_v[:, D:2 * D], preferred_element_type=f32).astype(bf16)
            for cc in range(BQ // C):
                c = qb * (BQ // C) + cc
                for b in range(BPC[c]):
                    r0 = cc * C + (BPC[c] - 1 - b) * 16
                    for g in range(4):
                        k_scr[g, pl.ds((MSTART[c] + b) * 8, 8), :] = pltpu.bitcast(
                            k[r0:r0 + 16, g * 128:(g + 1) * 128], u32)
                if RV[c]:
                    r0 = cc * C + RM[c]
                    kf = k[r0:r0 + RV[c]].astype(f32)
                    for g in range(4):
                        kv_scr[g, pl.ds(VSTART[c], RV[c]), :] = kf[:, g * 128:(g + 1) * 128]

        def proj_q(qb, xn, wq_t):
            qt = lax.dot_general(wq_t, xn, NT, preferred_element_type=f32)
            qt_scr[qb] = (qt * (DH ** -0.5 * LOG2E)).astype(bf16)

        def proj_v(qb, xn, wv_t):
            vt = lax.dot_general(wv_t, xn, NT, preferred_element_type=f32)
            vt_scr[:, :, pl.ds(qb * BQ, BQ)] = vt.astype(bf16).astype(f32).reshape(H, DH, BQ)

        def ln_chunk(qb):
            return _ln(x_v[pl.ds(qb * BQ, BQ), :].astype(f32)).astype(bf16)

        x_copy(0).wait()
        xn0 = ln_chunk(0)
        w_copy(1).wait()
        proj_k(0, xn0)
        w_copy(0).wait()
        w_copy(2).wait()
        wq_t = wqkv_v[:, 0:D].astype(f32).T.astype(bf16)
        wv_t = wqkv_v[:, 2 * D:3 * D].astype(f32).T.astype(bf16)
        proj_q(0, xn0, wq_t)
        for j in range(len(late)):
            late_copy(j).start()
        x_copy(1).wait()
        xn1 = ln_chunk(1)
        proj_v(0, xn0, wv_t)
        for i in range(2, NQ):
            x_copy(i).wait()
        for qb in range(1, NQ):
            xn = xn1 if qb == 1 else ln_chunk(qb)
            proj_k(qb, xn)
            proj_q(qb, xn, wq_t)
            proj_v(qb, xn, wv_t)
        produce_kb(0, kb_a)
        prep_q_first(0)

    @pl.when(step < NAS)
    def _():
        h0 = step * HPS
        items = [(u, qb) for u in range(HPS) for qb in range(NQ)]
        kbs = [kb_a, kb_b]
        qms, qbv, blk, acc, lacc, vout = {}, {}, {}, {}, {}, {}
        chunks = [(it, c) for it in range(len(items)) for c in range(NC)]
        vpieces = [(it, c, lt, hf) for (it, c) in chunks if RV[c] for lt in range(NLT) for hf in range(2)]
        st = {"bad": None, "vi": 0, "cur": None, "tok": None, "sid": 0}
        links = {}

        def add_bad(b):
            st["bad"] = b if st["bad"] is None else jnp.maximum(st["bad"], b)

        def emit_vpiece():
            if st["vi"] >= len(vpieces):
                return
            it, c, lt, hf = vpieces[st["vi"]]
            st["vi"] += 1
            u, qb = items[it]
            if it not in qbv:
                qbv[it] = [qb_first[d] for d in range(DH)] if it == 0 else q_bcast(h0 + u, qb)
            if hf == 0:
                st["sid"] = (st["vi"] // 2) % NTH
                lk = links.get(st["sid"])
                a = None if lk is None else lk - lk
            else:
                a = st["cur"]
            for d in range(hf * 8, hf * 8 + 8):
                kbd = kbs[u % 2][d, pl.ds(VSTART[c], RV[c]), :]
                qbb = jnp.concatenate([qbv[it][d][:, lt * 128:(lt + 1) * 128]] * (RV[c] // 8), axis=0)
                term = kbd * qbb
                a = term if a is None else a + term
            st["cur"] = a
            if hf == 1:
                vout.setdefault((it, c), []).append(a)
                links[st["sid"]] = a

        def sum_add(it, p16, j):
            s2 = p16[0:8] + p16[8:16]
            key = (it, j % 2)
            lacc[key] = s2 if key not in lacc else lacc[key] + s2

        def emit_pv(ci):
            it, c = chunks[ci]
            u, qb = items[it]
            if c == 3 and qb == 1:
                produce_kb(jnp.minimum(h0 + u + 1, H - 1), kbs[(u + 1) % 2])
            while RV[c] and len(vout.get((it, c), [])) < NLT:
                emit_vpiece()
            target = len([cc for cc in chunks[:ci + 1 + VAHEAD] if RV[cc[1]]]) * NLT * 2
            todo = max(target - st["vi"], 0)
            ps = []
            if RV[c]:
                pvv = jnp.exp2(jnp.concatenate(vout.pop((it, c)), axis=1))
                sum_add(it, pvv, 0)
            for b in range(BPC[c]):
                p16 = jnp.exp2(blk.pop((it, MSTART[c] + b)))
                sum_add(it, p16, b + 1)
                ps.append(p16)
                for _ in range((todo * (b + 1)) // BPC[c] - (todo * b) // BPC[c]):
                    emit_vpiece()
            ps = ps[::-1]
            if RV[c]:
                ps.append(pvv)
            p = jnp.concatenate(ps, axis=0)
            if ci == len(chunks) - 1:
                p_def[...] = p
                acc_def[...] = acc.pop(it)
                l_def[...] = lacc.pop((it, 0)) + lacc.pop((it, 1))
                return
            pv = _pv_dot(vt_scr[h0 + u, :, pl.ds(c * C, C)], p)
            z = pv[0:8, 0:128] - pv[0:8, 0:128]
            t = z if st["tok"] is None else st["tok"] + z
            st["tok"] = pltpu.roll(t, 1, 1) if TOKP[ci % len(TOKP)] == "r" else t
            acc[it] = pv if c == 0 else acc[it] + pv
            if c == NC - 1:
                o, bad = _normalise(acc.pop(it), lacc.pop((it, 0)) + lacc.pop((it, 1)))
                add_bad(bad)
                ot_scr[qb, pl.ds(pl.multiple_of((h0 + u) * DH, DH), DH), :] = o

        add_bad(deferred_pv(jnp.maximum(h0 - 1, 0)))
        pvi = 0
        for it, (u, qb) in enumerate(items):
            qms[it] = masked_qt(h0 + u, qb)
            bounds = sorted(set([0, NB] + [MSTART[c] + OFFB for c in range(NC) if MSTART[c] + OFFB < NB]))
            for a, b in zip(bounds[:-1], bounds[1:]):
                sm = jnp.dot(k_rows((h0 + u) // 8, a, b - a), qms[it], preferred_element_type=f32)
                for j in range(a, b):
                    blk[(it, j)] = sm[(j - a) * 16:(j - a + 1) * 16]
                pos = it * NB + b
                while pvi < len(chunks):
                    cit, cc = chunks[pvi]
                    nxt = cc + 2
                    need = cit * NB + MSTART[nxt] if nxt <= NC else (cit + 1) * NB + MSTART[nxt - NC]
                    if need + OFFB > pos:
                        break
                    emit_pv(pvi)
                    pvi += 1
        while pvi < len(chunks):
            emit_pv(pvi)
            pvi += 1
        prep_q_first(jnp.minimum(h0 + HPS, H - 1))
        tok_bad = jnp.where(st["tok"] == 0.0, 0.0, 1.0)
        add_bad(jnp.concatenate([tok_bad] * NLT, axis=1))
        bad_scr[...] = jnp.maximum(bad_scr[...], st["bad"])

    @pl.when(step == NAS)
    def _():
        for j in range(len(late)):
            late_copy(j).wait()
        bad = jnp.maximum(bad_scr[...], deferred_pv(H - 1))
        o_pre[...] = o_rows(0, 0)

        @pl.when(jnp.max(bad) > 0.0)
        def _():
            def body(i, carry):
                h = i // NQ
                qb = i % NQ
                qm = masked_qt(h, qb)
                sm = jnp.dot(k_rows(h // 8, 0, NB), qm, preferred_element_type=f32)
                sv = jnp.dot(kv_scr[h // 8].astype(bf16), qm, preferred_element_type=f32)
                m = jnp.maximum(jnp.max(sm, axis=0, keepdims=True), jnp.max(sv, axis=0, keepdims=True))
                pm = jnp.exp2(sm - m)
                pvv = jnp.exp2(sv - m)
                l = jnp.sum(pm, axis=0, keepdims=True) + jnp.sum(pvv, axis=0, keepdims=True)
                parts = []
                for c in range(NC):
                    for b in range(BPC[c]):
                        j = MSTART[c] + BPC[c] - 1 - b
                        parts.append(pm[j * 16:(j + 1) * 16])
                    if RV[c]:
                        parts.append(pvv[VSTART[c]:VSTART[c] + RV[c]])
                pn = jnp.concatenate(parts, axis=0)
                a = _pv_dot(vt_scr[h], pn)
                ot_scr[qb, pl.ds(pl.multiple_of(h * DH, DH), DH), :] = (a * (1.0 / l)).astype(bf16)
                return carry
            lax.fori_loop(0, H * NQ, body, 0)
            o_pre[...] = o_rows(0, 0)

    @pl.when(step >= NAS)
    def _():
        fb = step - NAS
        rng = range(FSUB)
        r0 = [pl.multiple_of(fb * BQ + j * SUB, SUB) for j in rng]
        o = [o_pre[...] if j == 0 else o_rows(fb, j) for j in rng]
        h1 = [x_v[pl.ds(r0[j], SUB), :].astype(f32) + jnp.dot(o[j], wo_v[...], preferred_element_type=f32)
              for j in rng]
        hn = [_ln(h1[j]).astype(bf16) for j in rng]
        act = []
        for j in rng:
            gate = lax.dot_general(w1t_v[...], hn[j], NT, preferred_element_type=f32)
            up = lax.dot_general(w3t_v[...], hn[j], NT, preferred_element_type=f32)
            act.append((gate * jax.nn.sigmoid(gate) * up).T.astype(bf16))
        for j in rng:
            out = h1[j] + jnp.dot(act[j], w2_v[...], preferred_element_type=f32)
            out_v[pl.ds(r0[j], SUB), :] = out.astype(bf16)
            out_copy(r0[j], fb * FSUB + j).start()
        o_pre[...] = o_rows(jnp.minimum(fb + 1, NQ - 1), 0)

    @pl.when(step == NAS + NQ - 1)
    def _():
        for i in range(NQ * FSUB):
            out_copy(i * SUB, i).wait()


@jax.jit
def pallas_sequential_preLN__softmax_full_mha__glu_gated_swiglu__prompt_kernel(
    A_x: jax.Array,
    A_wqkv: jax.Array,
    A_wo: jax.Array,
    B_x: jax.Array,
    B_w1: jax.Array,
    B_w3: jax.Array,
    B_w2: jax.Array,
):
    hbm = pl.BlockSpec(memory_space=pl.ANY)
    out = pl.pallas_call(
        _kernel,
        grid=(NAS + NQ,),
        in_specs=[hbm] * 6,
        out_specs=hbm,
        out_shape=jax.ShapeDtypeStruct((S, D), bf16),
        scratch_shapes=[
            pltpu.VMEM((S, D), bf16),
            pltpu.VMEM((D, 3 * D), bf16),
            pltpu.VMEM((D, D), bf16),
            pltpu.VMEM((F, D), bf16),
            pltpu.VMEM((F, D), bf16),
            pltpu.VMEM((F, D), bf16),
            pltpu.VMEM((S, D), bf16),
            pltpu.VMEM((4, NBP * 8, 128), u32),
            pltpu.VMEM((4, NV, 128), f32),
            pltpu.VMEM((NQ, D, BQ), bf16),
            pltpu.VMEM((H, DH, S), f32),
            pltpu.VMEM((NQ, D, BQ), bf16),
            pltpu.VMEM((8, BQ), f32),
            pltpu.VMEM((DH, NV, 128), f32),
            pltpu.VMEM((DH, NV, 128), f32),
            pltpu.VMEM((DH, 8, BQ), f32),
            pltpu.VMEM((C, BQ), f32),
            pltpu.VMEM((DH, BQ), f32),
            pltpu.VMEM((8, BQ), f32),
            pltpu.VMEM((SUB, D), bf16),
            pltpu.SemaphoreType.DMA((NQ + 3 + 4,)),
            pltpu.SemaphoreType.DMA((NQ * FSUB,)),
        ],
        compiler_params=pltpu.CompilerParams(dimension_semantics=("arbitrary",),
                                             vmem_limit_bytes=100 * 1024 * 1024),
    )(A_x.reshape(S, D), A_wqkv, A_wo, B_w1.T, B_w3.T, B_w2)
    return out.reshape(1, S, D)
```

```python
import jax
import jax.numpy as jnp
from jax import lax
from jax.experimental import pallas as pl
from jax.experimental.pallas import tpu as pltpu

S, D, H, DH, F = 2048, 512, 32, 16, 1376
LOG2E = 1.4426950408889634
EPS = 1e-5
f32, bf16, u32 = jnp.float32, jnp.bfloat16, jnp.uint32

BQ = 512
NQ = S // BQ
NLT = BQ // 128
C = 128
NC = S // C
HPS = 2
NAS = H // HPS
OFFB = 2
VAHEAD = 5
VPAT = (16,) * 15 + (0,)
NTH = 3
TOKP = "r-r"
FSUB = 4
SUB = BQ // FSUB
L_LO, L_HI, A_HI = 2.0 ** -40, 2.0 ** 100, 2.0 ** 120
NT = (((1,), (1,)), ((), ()))

RV = [VPAT[c % len(VPAT)] for c in range(NC)]
RM = [C - v for v in RV]
BPC = [r // 16 for r in RM]
MSTART = [sum(BPC[:c]) for c in range(NC + 1)]
VSTART = [sum(RV[:c]) for c in range(NC + 1)]
NB = MSTART[-1]
NBP = -(-NB // 4) * 4
NV = VSTART[-1]


def _ln(x):
    m = jnp.mean(x, axis=-1, keepdims=True)
    xc = x - m
    v = jnp.mean(xc * xc, axis=-1, keepdims=True)
    return xc * lax.rsqrt(v + EPS)


def _pv_dot(vt, p):
    return jnp.dot(vt, p, precision=lax.Precision.DEFAULT, preferred_element_type=f32)


def _normalise(a, l8):
    l = jnp.sum(l8, axis=0, keepdims=True)
    ok_l = jnp.logical_and(l >= L_LO, l <= L_HI)
    bad_a = jnp.where(jnp.abs(a) <= A_HI, 0.0, 1.0)
    bad = jnp.maximum(jnp.maximum(bad_a[0:8], bad_a[8:16]), jnp.where(ok_l, 0.0, 1.0))
    return (a * (1.0 / l)).astype(bf16), bad


def _kernel(x_hbm, wqkv_hbm, wo_hbm, w1t_hbm, w3t_hbm, w2_hbm, o_hbm,
            x_v, wq_v, wk_v, wv_v, wo_v, w1t_v, w3t_v, w2_v, out_v,
            k_scr, kv_scr, qt_scr, vt_scr, ot_scr, bad_scr, kb_a, kb_b, qb_first, p_def, acc_def, l_def, o_pre,
            sems, osems):
    step = pl.program_id(0)

    def x_copy(i):
        return pltpu.make_async_copy(x_hbm.at[pl.ds(i * BQ, BQ), :], x_v.at[i], sems.at[i])

    def w_copy(j):
        return pltpu.make_async_copy(wqkv_hbm.at[:, pl.ds(j * D, D)], (wq_v, wk_v, wv_v)[j], sems.at[NQ + j])

    late = [(wo_hbm, wo_v), (w1t_hbm, w1t_v), (w3t_hbm, w3t_v), (w2_hbm, w2_v)]

    def late_copy(j):
        return pltpu.make_async_copy(late[j][0], late[j][1], sems.at[NQ + 3 + j])

    def out_copy(i):
        return pltpu.make_async_copy(out_v.at[i], o_hbm.at[pl.ds(pl.multiple_of(i * SUB, SUB), SUB), :], osems.at[i])

    def k_rows(g, blk0, nblk):
        return pltpu.bitcast(k_scr[g, pl.ds(blk0 * 8, nblk * 8), :], bf16)

    def masked_qt(h, qb):
        qt = qt_scr[qb, pl.ds(pl.multiple_of((h // 8) * 128, 128), 128), :]
        rows = lax.broadcasted_iota(jnp.int32, (128, BQ), 0) // DH
        return jnp.where(rows == h % 8, qt.astype(f32), 0.0).astype(bf16)

    def produce_kb(h, kb):
        x = pltpu.roll(kv_scr[h // 8], (128 - (h % 8) * DH) % 128, 1)
        for d in range(DH):
            kb[d] = jnp.broadcast_to(x[:, d:d + 1], (NV, 128))

    def q_bcast(h, qb):
        q16 = qt_scr[qb, pl.ds(pl.multiple_of(h * DH, DH), DH), :].astype(f32)
        return [jnp.broadcast_to(q16[d:d + 1, :], (8, BQ)) for d in range(DH)]

    def prep_q_first(h):
        for d, v in enumerate(q_bcast(h, 0)):
            qb_first[d] = v

    def o_rows(fb, j):
        return ot_scr[fb, :, pl.ds(j * SUB, SUB)].astype(f32).T.astype(bf16)

    def deferred_pv(h):
        a = acc_def[...] + _pv_dot(vt_scr[h, :, pl.ds((NC - 1) * C, C)], p_def[...])
        o, bad = _normalise(a, l_def[...])
        ot_scr[NQ - 1, pl.ds(pl.multiple_of(h * DH, DH), DH), :] = o
        return bad

    @pl.when(step == 0)
    def _():
        x_copy(0).start()
        w_copy(1).start()
        w_copy(0).start()
        w_copy(2).start()
        for i in range(1, NQ):
            x_copy(i).start()
        bad_scr[...] = jnp.zeros_like(bad_scr)
        p_def[...] = jnp.zeros_like(p_def)
        acc_def[...] = jnp.zeros_like(acc_def)
        l_def[...] = jnp.ones_like(l_def)

        def proj_k(qb, xn):
            k = jnp.dot(xn, wk_v[...], preferred_element_type=f32).astype(bf16)
            for cc in range(BQ // C):
                c = qb * (BQ // C) + cc
                for b in range(BPC[c]):
                    r0 = cc * C + (BPC[c] - 1 - b) * 16
                    for g in range(4):
                        k_scr[g, pl.ds((MSTART[c] + b) * 8, 8), :] = pltpu.bitcast(
                            k[r0:r0 + 16, g * 128:(g + 1) * 128], u32)
                if RV[c]:
                    r0 = cc * C + RM[c]
                    kf = k[r0:r0 + RV[c]].astype(f32)
                    for g in range(4):
                        kv_scr[g, pl.ds(VSTART[c], RV[c]), :] = kf[:, g * 128:(g + 1) * 128]

        def proj_q(qb, xn, wq_t):
            qt = lax.dot_general(wq_t, xn, NT, preferred_element_type=f32)
            qt_scr[qb] = (qt * (DH ** -0.5 * LOG2E)).astype(bf16)

        def proj_v(qb, xn, wv_t):
            vt = lax.dot_general(wv_t, xn, NT, preferred_element_type=f32)
            vt_scr[:, :, pl.ds(qb * BQ, BQ)] = vt.astype(bf16).astype(f32).reshape(H, DH, BQ)

        def ln_chunk(qb):
            return _ln(x_v[qb].astype(f32)).astype(bf16)

        x_copy(0).wait()
        xn0 = ln_chunk(0)
        w_copy(1).wait()
        proj_k(0, xn0)
        w_copy(0).wait()
        w_copy(2).wait()
        wq_t = wq_v[...].astype(f32).T.astype(bf16)
        wv_t = wv_v[...].astype(f32).T.astype(bf16)
        proj_q(0, xn0, wq_t)
        for j in range(len(late)):
            late_copy(j).start()
        x_copy(1).wait()
        xn1 = ln_chunk(1)
        proj_v(0, xn0, wv_t)
        for i in range(2, NQ):
            x_copy(i).wait()
        for qb in range(1, NQ):
            xn = xn1 if qb == 1 else ln_chunk(qb)
            proj_k(qb, xn)
            proj_q(qb, xn, wq_t)
            proj_v(qb, xn, wv_t)
        produce_kb(0, kb_a)
        prep_q_first(0)

    @pl.when(step < NAS)
    def _():
        h0 = step * HPS
        items = [(u, qb) for u in range(HPS) for qb in range(NQ)]
        kbs = [kb_a, kb_b]
        qms, qbv, blk, acc, lacc, vout = {}, {}, {}, {}, {}, {}
        chunks = [(it, c) for it in range(len(items)) for c in range(NC)]
        vpieces = [(it, c, lt, hf) for (it, c) in chunks if RV[c] for lt in range(NLT) for hf in range(2)]
        st = {"bad": None, "vi": 0, "cur": None, "tok": None, "sid": 0}
        links = {}

        def add_bad(b):
            st["bad"] = b if st["bad"] is None else jnp.maximum(st["bad"], b)

        def emit_vpiece():
            if st["vi"] >= len(vpieces):
                return
            it, c, lt, hf = vpieces[st["vi"]]
            st["vi"] += 1
            u, qb = items[it]
            if it not in qbv:
                qbv[it] = [qb_first[d] for d in range(DH)] if it == 0 else q_bcast(h0 + u, qb)
            if hf == 0:
                st["sid"] = (st["vi"] // 2) % NTH
                lk = links.get(st["sid"])
                a = None if lk is None else lk - lk
            else:
                a = st["cur"]
            for d in range(hf * 8, hf * 8 + 8):
                kbd = kbs[u % 2][d, pl.ds(VSTART[c], RV[c]), :]
                qbb = jnp.concatenate([qbv[it][d][:, lt * 128:(lt + 1) * 128]] * (RV[c] // 8), axis=0)
                term = kbd * qbb
                a = term if a is None else a + term
            st["cur"] = a
            if hf == 1:
                vout.setdefault((it, c), []).append(a)
                links[st["sid"]] = a

        def sum_add(it, p16, j):
            s2 = p16[0:8] + p16[8:16]
            key = (it, j % 2)
            lacc[key] = s2 if key not in lacc else lacc[key] + s2

        def emit_pv(ci):
            it, c = chunks[ci]
            u, qb = items[it]
            if c == 3 and qb == 1:
                produce_kb(jnp.minimum(h0 + u + 1, H - 1), kbs[(u + 1) % 2])
            while RV[c] and len(vout.get((it, c), [])) < NLT:
                emit_vpiece()
            target = len([cc for cc in chunks[:ci + 1 + VAHEAD] if RV[cc[1]]]) * NLT * 2
            todo = max(target - st["vi"], 0)
            ps = []
            if RV[c]:
                pvv = jnp.exp2(jnp.concatenate(vout.pop((it, c)), axis=1))
                sum_add(it, pvv, 0)
            for b in range(BPC[c]):
                p16 = jnp.exp2(blk.pop((it, MSTART[c] + b)))
                sum_add(it, p16, b + 1)
                ps.append(p16)
                for _ in range((todo * (b + 1)) // BPC[c] - (todo * b) // BPC[c]):
                    emit_vpiece()
            ps = ps[::-1]
            if RV[c]:
                ps.append(pvv)
            p = jnp.concatenate(ps, axis=0)
            if ci == len(chunks) - 1:
                p_def[...] = p
                acc_def[...] = acc.pop(it)
                l_def[...] = lacc.pop((it, 0)) + lacc.pop((it, 1))
                return
            pv = _pv_dot(vt_scr[h0 + u, :, pl.ds(c * C, C)], p)
            z = pv[0:8, 0:128] - pv[0:8, 0:128]
            t = z if st["tok"] is None else st["tok"] + z
            st["tok"] = pltpu.roll(t, 1, 1) if TOKP[ci % len(TOKP)] == "r" else t
            acc[it] = pv if c == 0 else acc[it] + pv
            if c == NC - 1:
                o, bad = _normalise(acc.pop(it), lacc.pop((it, 0)) + lacc.pop((it, 1)))
                add_bad(bad)
                ot_scr[qb, pl.ds(pl.multiple_of((h0 + u) * DH, DH), DH), :] = o

        add_bad(deferred_pv(jnp.maximum(h0 - 1, 0)))
        pvi = 0
        for it, (u, qb) in enumerate(items):
            qms[it] = masked_qt(h0 + u, qb)
            bounds = sorted(set([0, NB] + [MSTART[c] + OFFB for c in range(NC) if MSTART[c] + OFFB < NB]))
            for a, b in zip(bounds[:-1], bounds[1:]):
                sm = jnp.dot(k_rows((h0 + u) // 8, a, b - a), qms[it], preferred_element_type=f32)
                for j in range(a, b):
                    blk[(it, j)] = sm[(j - a) * 16:(j - a + 1) * 16]
                pos = it * NB + b
                while pvi < len(chunks):
                    cit, cc = chunks[pvi]
                    nxt = cc + 2
                    need = cit * NB + MSTART[nxt] if nxt <= NC else (cit + 1) * NB + MSTART[nxt - NC]
                    if need + OFFB > pos:
                        break
                    emit_pv(pvi)
                    pvi += 1
        while pvi < len(chunks):
            emit_pv(pvi)
            pvi += 1
        prep_q_first(jnp.minimum(h0 + HPS, H - 1))
        tok_bad = jnp.where(st["tok"] == 0.0, 0.0, 1.0)
        add_bad(jnp.concatenate([tok_bad] * NLT, axis=1))
        bad_scr[...] = jnp.maximum(bad_scr[...], st["bad"])

    @pl.when(step == NAS)
    def _():
        for j in range(len(late)):
            late_copy(j).wait()
        bad = jnp.maximum(bad_scr[...], deferred_pv(H - 1))
        o_pre[...] = o_rows(0, 0)

        @pl.when(jnp.max(bad) > 0.0)
        def _():
            def body(i, carry):
                h = i // NQ
                qb = i % NQ
                qm = masked_qt(h, qb)
                sm = jnp.dot(k_rows(h // 8, 0, NB), qm, preferred_element_type=f32)
                sv = jnp.dot(kv_scr[h // 8].astype(bf16), qm, preferred_element_type=f32)
                m = jnp.maximum(jnp.max(sm, axis=0, keepdims=True), jnp.max(sv, axis=0, keepdims=True))
                pm = jnp.exp2(sm - m)
                pvv = jnp.exp2(sv - m)
                l = jnp.sum(pm, axis=0, keepdims=True) + jnp.sum(pvv, axis=0, keepdims=True)
                parts = []
                for c in range(NC):
                    for b in range(BPC[c]):
                        j = MSTART[c] + BPC[c] - 1 - b
                        parts.append(pm[j * 16:(j + 1) * 16])
                    if RV[c]:
                        parts.append(pvv[VSTART[c]:VSTART[c] + RV[c]])
                pn = jnp.concatenate(parts, axis=0)
                a = _pv_dot(vt_scr[h], pn)
                ot_scr[qb, pl.ds(pl.multiple_of(h * DH, DH), DH), :] = (a * (1.0 / l)).astype(bf16)
                return carry
            lax.fori_loop(0, H * NQ, body, 0)
            o_pre[...] = o_rows(0, 0)

    @pl.when(step >= NAS)
    def _():
        fb = step - NAS
        rng = range(FSUB)
        o = [o_pre[...] if j == 0 else o_rows(fb, j) for j in rng]
        h1 = [x_v[fb, pl.ds(j * SUB, SUB), :].astype(f32) + jnp.dot(o[j], wo_v[...], preferred_element_type=f32)
              for j in rng]
        hn = [_ln(h1[j]).astype(bf16) for j in rng]
        act = []
        for j in rng:
            gate = lax.dot_general(w1t_v[...], hn[j], NT, preferred_element_type=f32)
            up = lax.dot_general(w3t_v[...], hn[j], NT, preferred_element_type=f32)
            act.append((gate * jax.nn.sigmoid(gate) * up).T.astype(bf16))
        for j in rng:
            out = h1[j] + jnp.dot(act[j], w2_v[...], preferred_element_type=f32)
            out_v[fb * FSUB + j] = out.astype(bf16)
            out_copy(fb * FSUB + j).start()
        o_pre[...] = o_rows(jnp.minimum(fb + 1, NQ - 1), 0)

    @pl.when(step == NAS + NQ - 1)
    def _():
        for i in range(NQ * FSUB):
            out_copy(i).wait()


@jax.jit
def pallas_sequential_preLN__softmax_full_mha__glu_gated_swiglu__prompt_kernel(
    A_x: jax.Array,
    A_wqkv: jax.Array,
    A_wo: jax.Array,
    B_x: jax.Array,
    B_w1: jax.Array,
    B_w3: jax.Array,
    B_w2: jax.Array,
):
    hbm = pl.BlockSpec(memory_space=pl.ANY)
    out = pl.pallas_call(
        _kernel,
        grid=(NAS + NQ,),
        in_specs=[hbm] * 6,
        out_specs=hbm,
        out_shape=jax.ShapeDtypeStruct((S, D), bf16),
        scratch_shapes=[
            pltpu.VMEM((NQ, BQ, D), bf16),
            pltpu.VMEM((D, D), bf16),
            pltpu.VMEM((D, D), bf16),
            pltpu.VMEM((D, D), bf16),
            pltpu.VMEM((D, D), bf16),
            pltpu.VMEM((F, D), bf16),
            pltpu.VMEM((F, D), bf16),
            pltpu.VMEM((F, D), bf16),
            pltpu.VMEM((NQ * FSUB, SUB, D), bf16),
            pltpu.VMEM((4, NBP * 8, 128), u32),
            pltpu.VMEM((4, NV, 128), f32),
            pltpu.VMEM((NQ, D, BQ), bf16),
            pltpu.VMEM((H, DH, S), f32),
            pltpu.VMEM((NQ, D, BQ), bf16),
            pltpu.VMEM((8, BQ), f32),
            pltpu.VMEM((DH, NV, 128), f32),
            pltpu.VMEM((DH, NV, 128), f32),
            pltpu.VMEM((DH, 8, BQ), f32),
            pltpu.VMEM((C, BQ), f32),
            pltpu.VMEM((DH, BQ), f32),
            pltpu.VMEM((8, BQ), f32),
            pltpu.VMEM((SUB, D), bf16),
            pltpu.SemaphoreType.DMA((NQ + 3 + 4,)),
            pltpu.SemaphoreType.DMA((NQ * FSUB,)),
        ],
        compiler_params=pltpu.CompilerParams(dimension_semantics=("arbitrary",),
                                             vmem_limit_bytes=100 * 1024 * 1024),
    )(A_x.reshape(S, D), A_wqkv, A_wo, B_w1.T, B_w3.T, B_w2)
    return out.reshape(1, S, D)
```

```python
import jax
import jax.numpy as jnp
from jax import lax
from jax.experimental import pallas as pl
from jax.experimental.pallas import tpu as pltpu

S, D, H, DH, F = 2048, 512, 32, 16, 1376
LOG2E = 1.4426950408889634
EPS = 1e-5
f32, bf16, u32 = jnp.float32, jnp.bfloat16, jnp.uint32

BQ = 512
NQ = S // BQ
NLT = BQ // 128
C = 128
NC = S // C
HPS = 2
NAS = H // HPS
OFFB = 2
VAHEAD = 5
VPAT = (16,) * 5 + (32,) + (16,) * 5 + (32,) + (16,) * 3 + (0,)
NTH = 3
TOKP = "r-r"
FSUB = 4
SUB = BQ // FSUB
L_LO, L_HI, A_HI = 2.0 ** -40, 2.0 ** 100, 2.0 ** 120
NT = (((1,), (1,)), ((), ()))

RV = [VPAT[c % len(VPAT)] for c in range(NC)]
RM = [C - v for v in RV]
BPC = [r // 16 for r in RM]
MSTART = [sum(BPC[:c]) for c in range(NC + 1)]
VSTART = [sum(RV[:c]) for c in range(NC + 1)]
NB = MSTART[-1]
NBP = -(-NB // 4) * 4
NV = VSTART[-1]


def _ln(x):
    m = jnp.mean(x, axis=-1, keepdims=True)
    xc = x - m
    v = jnp.mean(xc * xc, axis=-1, keepdims=True)
    return xc * lax.rsqrt(v + EPS)


def _pv_dot(vt, p):
    return jnp.dot(vt, p, precision=lax.Precision.DEFAULT, preferred_element_type=f32)


def _normalise(a, l8):
    l = jnp.sum(l8, axis=0, keepdims=True)
    ok_l = jnp.logical_and(l >= L_LO, l <= L_HI)
    bad_a = jnp.where(jnp.abs(a) <= A_HI, 0.0, 1.0)
    bad = jnp.maximum(jnp.maximum(bad_a[0:8], bad_a[8:16]), jnp.where(ok_l, 0.0, 1.0))
    return (a * (1.0 / l)).astype(bf16), bad


def _kernel(x_hbm, wqkv_hbm, wo_hbm, w1t_hbm, w3t_hbm, w2_hbm, o_hbm,
            x_v, wq_v, wk_v, wv_v, wo_v, w1t_v, w3t_v, w2_v, out_v,
            k_all, kv_all, qt_scr, vt_scr, ot_scr, bad_scr, kb_a, kb_b, qb_first, p_def, acc_def, l_def, o_pre,
            sems, osems):
    step = pl.program_id(0)

    def x_copy(i):
        return pltpu.make_async_copy(x_hbm.at[pl.ds(i * BQ, BQ), :], x_v.at[i], sems.at[i])

    def w_copy(j):
        return pltpu.make_async_copy(wqkv_hbm.at[:, pl.ds(j * D, D)], (wq_v, wk_v, wv_v)[j], sems.at[NQ + j])

    late = [(wo_hbm, wo_v), (w1t_hbm, w1t_v), (w3t_hbm, w3t_v), (w2_hbm, w2_v)]

    def late_copy(j):
        return pltpu.make_async_copy(late[j][0], late[j][1], sems.at[NQ + 3 + j])

    def out_copy(i):
        return pltpu.make_async_copy(out_v.at[i], o_hbm.at[pl.ds(pl.multiple_of(i * SUB, SUB), SUB), :], osems.at[i])

    def k_rows(h, blk0, nblk):
        return pltpu.bitcast(k_all[h, pl.ds(blk0 * 8, nblk * 8), :], bf16)[:, 0:DH]

    def qt_rows(h, qb):
        return qt_scr[qb, pl.ds(pl.multiple_of(h * DH, DH), DH), :]

    def produce_kb(h, kb):
        x = kv_all[h]
        for d in range(DH):
            kb[d] = jnp.broadcast_to(x[:, d:d + 1], (NV, 128))

    def q_bcast(h, qb):
        q16 = qt_rows(h, qb).astype(f32)
        return [jnp.broadcast_to(q16[d:d + 1, :], (8, BQ)) for d in range(DH)]

    def prep_q_first(h):
        for d, v in enumerate(q_bcast(h, 0)):
            qb_first[d] = v

    def o_rows(fb, j):
        return ot_scr[fb, :, pl.ds(j * SUB, SUB)].astype(f32).T.astype(bf16)

    def deferred_pv(h):
        a = acc_def[...] + _pv_dot(vt_scr[h, :, pl.ds((NC - 1) * C, C)], p_def[...])
        o, bad = _normalise(a, l_def[...])
        ot_scr[NQ - 1, pl.ds(pl.multiple_of(h * DH, DH), DH), :] = o
        return bad

    @pl.when(step == 0)
    def _():
        x_copy(0).start()
        w_copy(1).start()
        w_copy(0).start()
        w_copy(2).start()
        for i in range(1, NQ):
            x_copy(i).start()
        bad_scr[...] = jnp.zeros_like(bad_scr)
        p_def[...] = jnp.zeros_like(p_def)
        acc_def[...] = jnp.zeros_like(acc_def)
        l_def[...] = jnp.ones_like(l_def)

        def proj_k(qb, xn):
            k = jnp.dot(xn, wk_v[...], preferred_element_type=f32).astype(bf16)
            for cc in range(BQ // C):
                c = qb * (BQ // C) + cc
                for b in range(BPC[c]):
                    r0 = cc * C + (BPC[c] - 1 - b) * 16
                    for g in range(4):
                        kw = pltpu.bitcast(k[r0:r0 + 16, g * 128:(g + 1) * 128], u32)
                        for hh in range(8):
                            k_all[g * 8 + hh, pl.ds((MSTART[c] + b) * 8, 8), :] = (
                                kw if hh == 0 else pltpu.roll(kw, 128 - hh * DH, 1))
                if RV[c]:
                    r0 = cc * C + RM[c]
                    kf = k[r0:r0 + RV[c]].astype(f32)
                    for g in range(4):
                        kfg = kf[:, g * 128:(g + 1) * 128]
                        for hh in range(8):
                            kv_all[g * 8 + hh, pl.ds(VSTART[c], RV[c]), :] = (
                                kfg if hh == 0 else pltpu.roll(kfg, 128 - hh * DH, 1))

        def proj_q(qb, xn, wq_t):
            qt = lax.dot_general(wq_t, xn, NT, preferred_element_type=f32)
            qt_scr[qb] = (qt * (DH ** -0.5 * LOG2E)).astype(bf16)

        def proj_v(qb, xn, wv_t):
            vt = lax.dot_general(wv_t, xn, NT, preferred_element_type=f32)
            vt_scr[:, :, pl.ds(qb * BQ, BQ)] = vt.astype(bf16).astype(f32).reshape(H, DH, BQ)

        def ln_chunk(qb):
            return _ln(x_v[qb].astype(f32)).astype(bf16)

        x_copy(0).wait()
        xn0 = ln_chunk(0)
        w_copy(1).wait()
        proj_k(0, xn0)
        w_copy(0).wait()
        w_copy(2).wait()
        wq_t = wq_v[...].astype(f32).T.astype(bf16)
        wv_t = wv_v[...].astype(f32).T.astype(bf16)
        proj_q(0, xn0, wq_t)
        for j in range(len(late)):
            late_copy(j).start()
        x_copy(1).wait()
        xn1 = ln_chunk(1)
        proj_v(0, xn0, wv_t)
        for i in range(2, NQ):
            x_copy(i).wait()
        for qb in range(1, NQ):
            xn = xn1 if qb == 1 else ln_chunk(qb)
            proj_k(qb, xn)
            proj_q(qb, xn, wq_t)
            proj_v(qb, xn, wv_t)
        produce_kb(0, kb_a)
        prep_q_first(0)

    @pl.when(step < NAS)
    def _():
        h0 = step * HPS
        items = [(u, qb) for u in range(HPS) for qb in range(NQ)]
        kbs = [kb_a, kb_b]
        qms, qbv, blk, acc, lacc, vout = {}, {}, {}, {}, {}, {}
        chunks = [(it, c) for it in range(len(items)) for c in range(NC)]
        vpieces = [(it, c, un, lt, hf) for (it, c) in chunks for un in range(RV[c] // 16)
                   for lt in range(NLT) for hf in range(2)]
        st = {"bad": None, "vi": 0, "cur": None, "tok": None, "sid": 0}
        links = {}

        def add_bad(b):
            st["bad"] = b if st["bad"] is None else jnp.maximum(st["bad"], b)

        def emit_vpiece():
            if st["vi"] >= len(vpieces):
                return
            it, c, un, lt, hf = vpieces[st["vi"]]
            st["vi"] += 1
            u, qb = items[it]
            if it not in qbv:
                qbv[it] = [qb_first[d] for d in range(DH)] if it == 0 else q_bcast(h0 + u, qb)
            if hf == 0:
                st["sid"] = (st["vi"] // 2) % NTH
                lk = links.get(st["sid"])
                a = None if lk is None else lk - lk
            else:
                a = st["cur"]
            for d in range(hf * 8, hf * 8 + 8):
                kbd = kbs[u % 2][d, pl.ds(VSTART[c] + un * 16, 16), :]
                qbb = jnp.concatenate([qbv[it][d][:, lt * 128:(lt + 1) * 128]] * 2, axis=0)
                term = kbd * qbb
                a = term if a is None else a + term
            st["cur"] = a
            if hf == 1:
                vout.setdefault((it, c), []).append(a)
                links[st["sid"]] = a

        def sum_add(it, p, j):
            s2 = p[0:8]
            for r in range(8, p.shape[0], 8):
                s2 = s2 + p[r:r + 8]
            key = (it, j % 2)
            lacc[key] = s2 if key not in lacc else lacc[key] + s2

        def emit_pv(ci):
            it, c = chunks[ci]
            u, qb = items[it]
            if c == 3 and qb == 1:
                produce_kb(jnp.minimum(h0 + u + 1, H - 1), kbs[(u + 1) % 2])
            while len(vout.get((it, c), [])) < NLT * (RV[c] // 16):
                emit_vpiece()
            target = sum(RV[cc[1]] // 16 for cc in chunks[:ci + 1 + VAHEAD]) * NLT * 2
            todo = max(target - st["vi"], 0)
            ps = []
            if RV[c]:
                vo = vout.pop((it, c))
                pvv = jnp.exp2(jnp.concatenate([jnp.concatenate(vo[un * NLT:(un + 1) * NLT], axis=1)
                                                for un in range(RV[c] // 16)], axis=0))
                sum_add(it, pvv, 0)
            for b in range(BPC[c]):
                p16 = jnp.exp2(blk.pop((it, MSTART[c] + b)))
                sum_add(it, p16, b + 1)
                ps.append(p16)
                for _ in range((todo * (b + 1)) // BPC[c] - (todo * b) // BPC[c]):
                    emit_vpiece()
            ps = ps[::-1]
            if RV[c]:
                ps.append(pvv)
            p = jnp.concatenate(ps, axis=0)
            if ci == len(chunks) - 1:
                p_def[...] = p
                acc_def[...] = acc.pop(it)
                l_def[...] = lacc.pop((it, 0)) + lacc.pop((it, 1))
                return
            pv = _pv_dot(vt_scr[h0 + u, :, pl.ds(c * C, C)], p)
            z = pv[0:8, 0:128] - pv[0:8, 0:128]
            t = z if st["tok"] is None else st["tok"] + z
            st["tok"] = pltpu.roll(t, 1, 1) if TOKP[ci % len(TOKP)] == "r" else t
            acc[it] = pv if c == 0 else acc[it] + pv
            if c == NC - 1:
                o, bad = _normalise(acc.pop(it), lacc.pop((it, 0)) + lacc.pop((it, 1)))
                add_bad(bad)
                ot_scr[qb, pl.ds(pl.multiple_of((h0 + u) * DH, DH), DH), :] = o

        add_bad(deferred_pv(jnp.maximum(h0 - 1, 0)))
        pvi = 0
        for it, (u, qb) in enumerate(items):
            qms[it] = qt_rows(h0 + u, qb)
            bounds = sorted(set([0, NB] + [MSTART[c] + OFFB for c in range(NC) if MSTART[c] + OFFB < NB]))
            for a, b in zip(bounds[:-1], bounds[1:]):
                sm = jnp.dot(k_rows(h0 + u, a, b - a), qms[it], preferred_element_type=f32)
                for j in range(a, b):
                    blk[(it, j)] = sm[(j - a) * 16:(j - a + 1) * 16]
                pos = it * NB + b
                while pvi < len(chunks):
                    cit, cc = chunks[pvi]
                    nxt = cc + 2
                    need = cit * NB + MSTART[nxt] if nxt <= NC else (cit + 1) * NB + MSTART[nxt - NC]
                    if need + OFFB > pos:
                        break
                    emit_pv(pvi)
                    pvi += 1
        while pvi < len(chunks):
            emit_pv(pvi)
            pvi += 1
        prep_q_first(jnp.minimum(h0 + HPS, H - 1))
        tok_bad = jnp.where(st["tok"] == 0.0, 0.0, 1.0)
        add_bad(jnp.concatenate([tok_bad] * NLT, axis=1))
        bad_scr[...] = jnp.maximum(bad_scr[...], st["bad"])

    @pl.when(step == NAS)
    def _():
        for j in range(len(late)):
            late_copy(j).wait()
        bad = jnp.maximum(bad_scr[...], deferred_pv(H - 1))
        o_pre[...] = o_rows(0, 0)

        @pl.when(jnp.max(bad) > 0.0)
        def _():
            def body(i, carry):
                h = i // NQ
                qb = i % NQ
                qm = qt_rows(h, qb)
                sm = jnp.dot(k_rows(h, 0, NB), qm, preferred_element_type=f32)
                sv = jnp.dot(kv_all[h][:, 0:DH].astype(bf16), qm, preferred_element_type=f32)
                m = jnp.maximum(jnp.max(sm, axis=0, keepdims=True), jnp.max(sv, axis=0, keepdims=True))
                pm = jnp.exp2(sm - m)
                pvv = jnp.exp2(sv - m)
                l = jnp.sum(pm, axis=0, keepdims=True) + jnp.sum(pvv, axis=0, keepdims=True)
                parts = []
                for c in range(NC):
                    for b in range(BPC[c]):
                        j = MSTART[c] + BPC[c] - 1 - b
                        parts.append(pm[j * 16:(j + 1) * 16])
                    if RV[c]:
                        parts.append(pvv[VSTART[c]:VSTART[c] + RV[c]])
                pn = jnp.concatenate(parts, axis=0)
                a = _pv_dot(vt_scr[h], pn)
                ot_scr[qb, pl.ds(pl.multiple_of(h * DH, DH), DH), :] = (a * (1.0 / l)).astype(bf16)
                return carry
            lax.fori_loop(0, H * NQ, body, 0)
            o_pre[...] = o_rows(0, 0)

    @pl.when(step >= NAS)
    def _():
        fb = step - NAS
        rng = range(FSUB)
        o = [o_pre[...] if j == 0 else o_rows(fb, j) for j in rng]
        h1 = [x_v[fb, pl.ds(j * SUB, SUB), :].astype(f32) + jnp.dot(o[j], wo_v[...], preferred_element_type=f32)
              for j in rng]
        hn = [_ln(h1[j]).astype(bf16) for j in rng]
        act = []
        for j in rng:
            gate = lax.dot_general(w1t_v[...], hn[j], NT, preferred_element_type=f32)
            up = lax.dot_general(w3t_v[...], hn[j], NT, preferred_element_type=f32)
            act.append((gate * jax.nn.sigmoid(gate) * up).T.astype(bf16))
        for j in rng:
            out = h1[j] + jnp.dot(act[j], w2_v[...], preferred_element_type=f32)
            out_v[fb * FSUB + j] = out.astype(bf16)
            out_copy(fb * FSUB + j).start()
        o_pre[...] = o_rows(jnp.minimum(fb + 1, NQ - 1), 0)

    @pl.when(step == NAS + NQ - 1)
    def _():
        for i in range(NQ * FSUB):
            out_copy(i).wait()


@jax.jit
def pallas_sequential_preLN__softmax_full_mha__glu_gated_swiglu__prompt_kernel(
    A_x: jax.Array,
    A_wqkv: jax.Array,
    A_wo: jax.Array,
    B_x: jax.Array,
    B_w1: jax.Array,
    B_w3: jax.Array,
    B_w2: jax.Array,
):
    hbm = pl.BlockSpec(memory_space=pl.ANY)
    out = pl.pallas_call(
        _kernel,
        grid=(NAS + NQ,),
        in_specs=[hbm] * 6,
        out_specs=hbm,
        out_shape=jax.ShapeDtypeStruct((S, D), bf16),
        scratch_shapes=[
            pltpu.VMEM((NQ, BQ, D), bf16),
            pltpu.VMEM((D, D), bf16),
            pltpu.VMEM((D, D), bf16),
            pltpu.VMEM((D, D), bf16),
            pltpu.VMEM((D, D), bf16),
            pltpu.VMEM((F, D), bf16),
            pltpu.VMEM((F, D), bf16),
            pltpu.VMEM((F, D), bf16),
            pltpu.VMEM((NQ * FSUB, SUB, D), bf16),
            pltpu.VMEM((H, NBP * 8, 128), u32),
            pltpu.VMEM((H, NV, 128), f32),
            pltpu.VMEM((NQ, D, BQ), bf16),
            pltpu.VMEM((H, DH, S), f32),
            pltpu.VMEM((NQ, D, BQ), bf16),
            pltpu.VMEM((8, BQ), f32),
            pltpu.VMEM((DH, NV, 128), f32),
            pltpu.VMEM((DH, NV, 128), f32),
            pltpu.VMEM((DH, 8, BQ), f32),
            pltpu.VMEM((C, BQ), f32),
            pltpu.VMEM((DH, BQ), f32),
            pltpu.VMEM((8, BQ), f32),
            pltpu.VMEM((SUB, D), bf16),
            pltpu.SemaphoreType.DMA((NQ + 3 + 4,)),
            pltpu.SemaphoreType.DMA((NQ * FSUB,)),
        ],
        compiler_params=pltpu.CompilerParams(dimension_semantics=("arbitrary",),
                                             vmem_limit_bytes=100 * 1024 * 1024),
    )(A_x.reshape(S, D), A_wqkv, A_wo, B_w1.T, B_w3.T, B_w2)
    return out.reshape(1, S, D)
```

```python
import jax
import jax.numpy as jnp
from jax import lax
from jax.experimental import pallas as pl
from jax.experimental.pallas import tpu as pltpu

S, D, H, DH, F = 2048, 512, 32, 16, 1376
LOG2E = 1.4426950408889634
EPS = 1e-5
f32, bf16, u32 = jnp.float32, jnp.bfloat16, jnp.uint32

BQ = 512
NQ = S // BQ
NLT = BQ // 128
C = 128
NC = S // C
HPS = 2
NAS = H // HPS
OFFB = 2
VAHEAD = 5
VPAT = (16,) * 5 + (32,) + (16,) * 5 + (32,) + (16,) * 3 + (0,)
NTH = 3
TOKP = "r-r"
FSUB = 4
SUB = BQ // FSUB
L_LO, L_HI, A_HI = 2.0 ** -40, 2.0 ** 100, 2.0 ** 120
NT = (((1,), (1,)), ((), ()))

RV = [VPAT[c % len(VPAT)] for c in range(NC)]
RM = [C - v for v in RV]
BPC = [r // 16 for r in RM]
MSTART = [sum(BPC[:c]) for c in range(NC + 1)]
VSTART = [sum(RV[:c]) for c in range(NC + 1)]
NB = MSTART[-1]
NBP = -(-NB // 4) * 4
NV = VSTART[-1]


def _ln(x):
    m = jnp.mean(x, axis=-1, keepdims=True)
    xc = x - m
    v = jnp.mean(xc * xc, axis=-1, keepdims=True)
    return xc * lax.rsqrt(v + EPS)


def _pv_dot(vt, p):
    return jnp.dot(vt, p, precision=lax.Precision.DEFAULT, preferred_element_type=f32)


def _normalise(a, l8):
    l = jnp.sum(l8, axis=0, keepdims=True)
    ok_l = jnp.logical_and(l >= L_LO, l <= L_HI)
    bad_a = jnp.where(jnp.abs(a) <= A_HI, 0.0, 1.0)
    bad = jnp.maximum(jnp.maximum(bad_a[0:8], bad_a[8:16]), jnp.where(ok_l, 0.0, 1.0))
    return (a * (1.0 / l)).astype(bf16), bad


def _kernel(x_hbm, wqkv_hbm, wo_hbm, w1t_hbm, w3t_hbm, w2_hbm, o_hbm,
            x_v, wq_v, wk_v, wv_v, wo_v, w1t_v, w3t_v, w2_v, out_v,
            k_all, kv_all, qt_scr, vt_scr, ot_scr, bad_scr, kb_a, kb_b, qb_first, p_def, acc_def, l_def, o_pre,
            sems, osems):
    step = pl.program_id(0)

    def x_copy(i):
        return pltpu.make_async_copy(x_hbm.at[pl.ds(i * BQ, BQ), :], x_v.at[i], sems.at[i])

    def w_copy(j):
        return pltpu.make_async_copy(wqkv_hbm.at[:, pl.ds(j * D, D)], (wq_v, wk_v, wv_v)[j], sems.at[NQ + j])

    late = [(wo_hbm, wo_v), (w1t_hbm, w1t_v), (w3t_hbm, w3t_v), (w2_hbm, w2_v)]

    def late_copy(j):
        return pltpu.make_async_copy(late[j][0], late[j][1], sems.at[NQ + 3 + j])

    def out_copy(i):
        return pltpu.make_async_copy(out_v.at[i], o_hbm.at[pl.ds(pl.multiple_of(i * SUB, SUB), SUB), :], osems.at[i])

    def k_rows(h, blk0, nblk):
        return pltpu.bitcast(k_all[h, pl.ds(blk0 * 8, nblk * 8), :], bf16)[:, 0:DH]

    def qt_rows(h, qb):
        return qt_scr[qb, pl.ds(pl.multiple_of(h * DH, DH), DH), :]

    def produce_kb(h, kb):
        x = kv_all[h]
        for d in range(DH):
            kb[d] = jnp.broadcast_to(x[:, d:d + 1], (NV, 128))

    def q_bcast(h, qb):
        q16 = qt_rows(h, qb).astype(f32)
        return [jnp.broadcast_to(q16[d:d + 1, :], (8, BQ)) for d in range(DH)]

    def prep_q_first(h):
        for d, v in enumerate(q_bcast(h, 0)):
            qb_first[d] = v

    def o_rows(fb, j):
        return ot_scr[fb, :, pl.ds(j * SUB, SUB)].astype(f32).T.astype(bf16)

    def deferred_pv(h):
        a = acc_def[...] + _pv_dot(vt_scr[h, :, pl.ds((NC - 1) * C, C)], p_def[...])
        o, bad = _normalise(a, l_def[...])
        ot_scr[NQ - 1, pl.ds(pl.multiple_of(h * DH, DH), DH), :] = o
        return bad

    @pl.when(step == 0)
    def _():
        x_copy(0).start()
        w_copy(1).start()
        w_copy(0).start()
        w_copy(2).start()
        for i in range(1, NQ):
            x_copy(i).start()
        bad_scr[...] = jnp.zeros_like(bad_scr)
        p_def[...] = jnp.zeros_like(p_def)
        acc_def[...] = jnp.zeros_like(acc_def)
        l_def[...] = jnp.ones_like(l_def)

        def proj_k(qb, xn, nrot=8):
            k = jnp.dot(xn, wk_v[...], preferred_element_type=f32).astype(bf16)
            for cc in range(BQ // C):
                c = qb * (BQ // C) + cc
                for b in range(BPC[c]):
                    r0 = cc * C + (BPC[c] - 1 - b) * 16
                    for g in range(4):
                        kw = pltpu.bitcast(k[r0:r0 + 16, g * 128:(g + 1) * 128], u32)
                        for hh in range(nrot):
                            k_all[g * 8 + hh, pl.ds((MSTART[c] + b) * 8, 8), :] = (
                                kw if hh == 0 else pltpu.roll(kw, 128 - hh * DH, 1))
                if RV[c]:
                    r0 = cc * C + RM[c]
                    kf = k[r0:r0 + RV[c]].astype(f32)
                    for g in range(4):
                        kfg = kf[:, g * 128:(g + 1) * 128]
                        for hh in range(nrot):
                            kv_all[g * 8 + hh, pl.ds(VSTART[c], RV[c]), :] = (
                                kfg if hh == 0 else pltpu.roll(kfg, 128 - hh * DH, 1))

        def proj_q(qb, xn, wq_t):
            qt = lax.dot_general(wq_t, xn, NT, preferred_element_type=f32)
            qt_scr[qb] = (qt * (DH ** -0.5 * LOG2E)).astype(bf16)

        def proj_v(qb, xn, wv_t):
            vt = lax.dot_general(wv_t, xn, NT, preferred_element_type=f32)
            vt_scr[:, :, pl.ds(qb * BQ, BQ)] = vt.astype(bf16).astype(f32).reshape(H, DH, BQ)

        def ln_chunk(qb):
            return _ln(x_v[qb].astype(f32)).astype(bf16)

        x_copy(0).wait()
        xn0 = ln_chunk(0)
        w_copy(1).wait()
        proj_k(0, xn0, nrot=1)
        w_copy(0).wait()
        w_copy(2).wait()
        wq_t = wq_v[...].astype(f32).T.astype(bf16)
        wv_t = wv_v[...].astype(f32).T.astype(bf16)
        proj_q(0, xn0, wq_t)
        for j in range(len(late)):
            late_copy(j).start()
        x_copy(1).wait()
        xn1 = ln_chunk(1)
        proj_v(0, xn0, wv_t)
        for i in range(2, NQ):
            x_copy(i).wait()
        nb0, nv0 = MSTART[BQ // C], VSTART[BQ // C]
        for g in range(4):
            kw = k_all[g * 8, pl.ds(0, nb0 * 8), :]
            kf = kv_all[g * 8, pl.ds(0, nv0), :]
            for hh in range(1, 8):
                k_all[g * 8 + hh, pl.ds(0, nb0 * 8), :] = pltpu.roll(kw, 128 - hh * DH, 1)
                kv_all[g * 8 + hh, pl.ds(0, nv0), :] = pltpu.roll(kf, 128 - hh * DH, 1)
        for qb in range(1, NQ):
            xn = xn1 if qb == 1 else ln_chunk(qb)
            proj_k(qb, xn)
            proj_q(qb, xn, wq_t)
            proj_v(qb, xn, wv_t)
        produce_kb(0, kb_a)
        prep_q_first(0)

    @pl.when(step < NAS)
    def _():
        h0 = step * HPS
        items = [(u, qb) for u in range(HPS) for qb in range(NQ)]
        kbs = [kb_a, kb_b]
        qms, qbv, blk, acc, lacc, vout = {}, {}, {}, {}, {}, {}
        chunks = [(it, c) for it in range(len(items)) for c in range(NC)]
        vpieces = [(it, c, un, lt, hf) for (it, c) in chunks for un in range(RV[c] // 16)
                   for lt in range(NLT) for hf in range(2)]
        st = {"bad": None, "vi": 0, "cur": None, "tok": None, "sid": 0}
        links = {}

        def add_bad(b):
            st["bad"] = b if st["bad"] is None else jnp.maximum(st["bad"], b)

        def emit_vpiece():
            if st["vi"] >= len(vpieces):
                return
            it, c, un, lt, hf = vpieces[st["vi"]]
            st["vi"] += 1
            u, qb = items[it]
            if it not in qbv:
                qbv[it] = [qb_first[d] for d in range(DH)] if it == 0 else q_bcast(h0 + u, qb)
            if hf == 0:
                st["sid"] = (st["vi"] // 2) % NTH
                lk = links.get(st["sid"])
                a = None if lk is None else lk - lk
            else:
                a = st["cur"]
            for d in range(hf * 8, hf * 8 + 8):
                kbd = kbs[u % 2][d, pl.ds(VSTART[c] + un * 16, 16), :]
                qbb = jnp.concatenate([qbv[it][d][:, lt * 128:(lt + 1) * 128]] * 2, axis=0)
                term = kbd * qbb
                a = term if a is None else a + term
            st["cur"] = a
            if hf == 1:
                vout.setdefault((it, c), []).append(a)
                links[st["sid"]] = a

        def sum_add(it, p, j):
            s2 = p[0:8]
            for r in range(8, p.shape[0], 8):
                s2 = s2 + p[r:r + 8]
            key = (it, j % 2)
            lacc[key] = s2 if key not in lacc else lacc[key] + s2

        def emit_pv(ci):
            it, c = chunks[ci]
            u, qb = items[it]
            if c == 3 and qb == 1:
                produce_kb(jnp.minimum(h0 + u + 1, H - 1), kbs[(u + 1) % 2])
            while len(vout.get((it, c), [])) < NLT * (RV[c] // 16):
                emit_vpiece()
            target = sum(RV[cc[1]] // 16 for cc in chunks[:ci + 1 + VAHEAD]) * NLT * 2
            todo = max(target - st["vi"], 0)
            ps = []
            if RV[c]:
                vo = vout.pop((it, c))
                pvv = jnp.exp2(jnp.concatenate([jnp.concatenate(vo[un * NLT:(un + 1) * NLT], axis=1)
                                                for un in range(RV[c] // 16)], axis=0))
                sum_add(it, pvv, 0)
            for b in range(BPC[c]):
                p16 = jnp.exp2(blk.pop((it, MSTART[c] + b)))
                sum_add(it, p16, b + 1)
                ps.append(p16)
                for _ in range((todo * (b + 1)) // BPC[c] - (todo * b) // BPC[c]):
                    emit_vpiece()
            ps = ps[::-1]
            if RV[c]:
                ps.append(pvv)
            p = jnp.concatenate(ps, axis=0)
            if ci == len(chunks) - 1:
                p_def[...] = p
                acc_def[...] = acc.pop(it)
                l_def[...] = lacc.pop((it, 0)) + lacc.pop((it, 1))
                return
            pv = _pv_dot(vt_scr[h0 + u, :, pl.ds(c * C, C)], p)
            z = pv[0:8, 0:128] - pv[0:8, 0:128]
            t = z if st["tok"] is None else st["tok"] + z
            st["tok"] = pltpu.roll(t, 1, 1) if TOKP[ci % len(TOKP)] == "r" else t
            acc[it] = pv if c == 0 else acc[it] + pv
            if c == NC - 1:
                o, bad = _normalise(acc.pop(it), lacc.pop((it, 0)) + lacc.pop((it, 1)))
                add_bad(bad)
                ot_scr[qb, pl.ds(pl.multiple_of((h0 + u) * DH, DH), DH), :] = o

        add_bad(deferred_pv(jnp.maximum(h0 - 1, 0)))
        pvi = 0
        for it, (u, qb) in enumerate(items):
            qms[it] = qt_rows(h0 + u, qb)
            bounds = sorted(set([0, NB] + [MSTART[c] + OFFB for c in range(1, NC) if MSTART[c] + OFFB < NB]))
            for a, b in zip(bounds[:-1], bounds[1:]):
                sm = jnp.dot(k_rows(h0 + u, a, b - a), qms[it], preferred_element_type=f32)
                for j in range(a, b):
                    blk[(it, j)] = sm[(j - a) * 16:(j - a + 1) * 16]
                pos = it * NB + b
                while pvi < len(chunks):
                    cit, cc = chunks[pvi]
                    nxt = cc + 2
                    need = cit * NB + MSTART[nxt] if nxt <= NC else (cit + 1) * NB + MSTART[nxt - NC]
                    if need + OFFB > pos:
                        break
                    emit_pv(pvi)
                    pvi += 1
        while pvi < len(chunks):
            emit_pv(pvi)
            pvi += 1
        prep_q_first(jnp.minimum(h0 + HPS, H - 1))
        tok_bad = jnp.where(st["tok"] == 0.0, 0.0, 1.0)
        add_bad(jnp.concatenate([tok_bad] * NLT, axis=1))
        bad_scr[...] = jnp.maximum(bad_scr[...], st["bad"])

    @pl.when(step == NAS)
    def _():
        for j in range(len(late)):
            late_copy(j).wait()
        bad = jnp.maximum(bad_scr[...], deferred_pv(H - 1))
        o_pre[...] = o_rows(0, 0)

        @pl.when(jnp.max(bad) > 0.0)
        def _():
            def body(i, carry):
                h = i // NQ
                qb = i % NQ
                qm = qt_rows(h, qb)
                sm = jnp.dot(k_rows(h, 0, NB), qm, preferred_element_type=f32)
                sv = jnp.dot(kv_all[h][:, 0:DH].astype(bf16), qm, preferred_element_type=f32)
                m = jnp.maximum(jnp.max(sm, axis=0, keepdims=True), jnp.max(sv, axis=0, keepdims=True))
                pm = jnp.exp2(sm - m)
                pvv = jnp.exp2(sv - m)
                l = jnp.sum(pm, axis=0, keepdims=True) + jnp.sum(pvv, axis=0, keepdims=True)
                parts = []
                for c in range(NC):
                    for b in range(BPC[c]):
                        j = MSTART[c] + BPC[c] - 1 - b
                        parts.append(pm[j * 16:(j + 1) * 16])
                    if RV[c]:
                        parts.append(pvv[VSTART[c]:VSTART[c] + RV[c]])
                pn = jnp.concatenate(parts, axis=0)
                a = _pv_dot(vt_scr[h], pn)
                ot_scr[qb, pl.ds(pl.multiple_of(h * DH, DH), DH), :] = (a * (1.0 / l)).astype(bf16)
                return carry
            lax.fori_loop(0, H * NQ, body, 0)
            o_pre[...] = o_rows(0, 0)

    @pl.when(step >= NAS)
    def _():
        fb = step - NAS
        rng = range(FSUB)
        o = [o_pre[...] if j == 0 else o_rows(fb, j) for j in rng]
        h1 = [x_v[fb, pl.ds(j * SUB, SUB), :].astype(f32) + jnp.dot(o[j], wo_v[...], preferred_element_type=f32)
              for j in rng]
        hn = [_ln(h1[j]).astype(bf16) for j in rng]
        act = []
        for j in rng:
            gate = lax.dot_general(w1t_v[...], hn[j], NT, preferred_element_type=f32)
            up = lax.dot_general(w3t_v[...], hn[j], NT, preferred_element_type=f32)
            act.append((gate * jax.nn.sigmoid(gate) * up).T.astype(bf16))
        for j in rng:
            out = h1[j] + jnp.dot(act[j], w2_v[...], preferred_element_type=f32)
            out_v[fb * FSUB + j] = out.astype(bf16)
            out_copy(fb * FSUB + j).start()
        o_pre[...] = o_rows(jnp.minimum(fb + 1, NQ - 1), 0)

    @pl.when(step == NAS + NQ - 1)
    def _():
        for i in range(NQ * FSUB):
            out_copy(i).wait()


@jax.jit
def pallas_sequential_preLN__softmax_full_mha__glu_gated_swiglu__prompt_kernel(
    A_x: jax.Array,
    A_wqkv: jax.Array,
    A_wo: jax.Array,
    B_x: jax.Array,
    B_w1: jax.Array,
    B_w3: jax.Array,
    B_w2: jax.Array,
):
    hbm = pl.BlockSpec(memory_space=pl.ANY)
    out = pl.pallas_call(
        _kernel,
        grid=(NAS + NQ,),
        in_specs=[hbm] * 6,
        out_specs=hbm,
        out_shape=jax.ShapeDtypeStruct((S, D), bf16),
        scratch_shapes=[
            pltpu.VMEM((NQ, BQ, D), bf16),
            pltpu.VMEM((D, D), bf16),
            pltpu.VMEM((D, D), bf16),
            pltpu.VMEM((D, D), bf16),
            pltpu.VMEM((D, D), bf16),
            pltpu.VMEM((F, D), bf16),
            pltpu.VMEM((F, D), bf16),
            pltpu.VMEM((F, D), bf16),
            pltpu.VMEM((NQ * FSUB, SUB, D), bf16),
            pltpu.VMEM((H, NBP * 8, 128), u32),
            pltpu.VMEM((H, NV, 128), f32),
            pltpu.VMEM((NQ, D, BQ), bf16),
            pltpu.VMEM((H, DH, S), f32),
            pltpu.VMEM((NQ, D, BQ), bf16),
            pltpu.VMEM((8, BQ), f32),
            pltpu.VMEM((DH, NV, 128), f32),
            pltpu.VMEM((DH, NV, 128), f32),
            pltpu.VMEM((DH, 8, BQ), f32),
            pltpu.VMEM((C, BQ), f32),
            pltpu.VMEM((DH, BQ), f32),
            pltpu.VMEM((8, BQ), f32),
            pltpu.VMEM((SUB, D), bf16),
            pltpu.SemaphoreType.DMA((NQ + 3 + 4,)),
            pltpu.SemaphoreType.DMA((NQ * FSUB,)),
        ],
        compiler_params=pltpu.CompilerParams(dimension_semantics=("arbitrary",),
                                             vmem_limit_bytes=100 * 1024 * 1024),
    )(A_x.reshape(S, D), A_wqkv, A_wo, B_w1.T, B_w3.T, B_w2)
    return out.reshape(1, S, D)
```
